```python
import os as _os
_os.environ.setdefault("JAX_PLATFORMS", "cpu")
import jax
import jax.numpy as jnp

def _softmax(x, axis=-1):
    return jax.nn.softmax(x, axis=axis)
def _gelu(x):
    return jax.nn.gelu(x, approximate=True)
def _silu(x):
    return jax.nn.silu(x)
def _sigmoid(x):
    return jax.nn.sigmoid(x)
def _layernorm(x, axis=-1, eps=1e-5):
    m = jnp.mean(x, axis=axis, keepdims=True)
    v = jnp.var(x, axis=axis, keepdims=True)
    return (x - m) / jnp.sqrt(v + eps)
def _scatter_add(tgt, idx, src, axis=0):
    return tgt.at[idx].add(src)
def _segment_sum(src, seg, n):
    return jax.ops.segment_sum(src, seg, n)
class _Rng:
    def __init__(self, key):
        self._k = key
    def _next(self):
        self._k, sub = jax.random.split(self._k)
        return sub
    def normal(self, shape):
        return jax.random.normal(self._next(), shape, dtype=jnp.bfloat16)
    def randint(self, lo, hi, shape):
        return jax.random.randint(self._next(), shape, lo, hi, dtype=jnp.int32)
    def uniform(self, shape, lo=0.0, hi=1.0):
        return jax.random.uniform(self._next(), shape, jnp.bfloat16, lo, hi)
    def permutation(self, n):
        return jax.random.permutation(self._next(), n)


kernel_name = 'gated_mix__linear_attn_block__mixer_s_mlp__prompt'

def setup_inputs():
    _rng = _Rng(jax.random.key(int.from_bytes(__import__("os").urandom(4), "little")))
    _w = (lambda a: (lambda t: t.astype(jnp.bfloat16) if jnp.issubdtype(t.dtype, jnp.floating) else t)(jnp.asarray(a)))
    def _A_setup():
        B, S, D = 1, 2048, 640
        return {
            "x": _w((lambda *s: _rng.normal(s) * 0.05)(B, S, D)),
            "wqkv": _w((lambda *s: _rng.normal(s) * 0.8)(D, 3 * D)),
            "wo": _w((lambda *s: _rng.normal(s) * 0.1)(D, D)),
        }
    _A_in = _A_setup()

    def _B_setup():
        B, S, D, F = 1, 2048, 640, 1728
        return {
            "x":  _w((lambda *s: _rng.normal(s) * 0.05)(B, S, D)),
            "w1": _w((lambda *s: _rng.normal(s) * 0.2)(D, D) * (D ** -0.5)),
            "w2": _w((lambda *s: _rng.normal(s) * 0.2)(D, D) * (D ** -0.5)),
            "w3": _w((lambda *s: _rng.normal(s) * 0.2)(D, F) * (D ** -0.5)),
            "w4": _w((lambda *s: _rng.normal(s) * 0.2)(F, D) * (F ** -0.5)),
        }
    _B_in = _B_setup()

    return {
        "A_x": _A_in["x"],
        "A_wqkv": _A_in["wqkv"],
        "A_wo": _A_in["wo"],
        "B_x": _B_in["x"],
        "B_w1": _B_in["w1"],
        "B_w2": _B_in["w2"],
        "B_w3": _B_in["w3"],
        "B_w4": _B_in["w4"],
        "gate_w": _w((lambda *s: _rng.normal(s) * 0.05)(640) * 16.0),
    }

def reference(A_x, A_wqkv, A_wo, B_x, B_w1, B_w2, B_w3, B_w4, gate_w):
    def _A_ref(x, wqkv, wo):
        B, S, D = x.shape
        H = 32; Dh = D // H
        qkv = (lambda x, *d: x.transpose(*d))((x @ wqkv).reshape(B, S, 3, H, Dh), 2, 0, 3, 1, 4)
        q, k, v = qkv[0], qkv[1], qkv[2]
        phi = lambda t: jnp.where(t > 0, t + 1, jnp.exp(t)) + 1e-6
        pq, pk = phi(q), phi(k)
        kv = jnp.einsum("bhsd,bhse->bhde", pk, v)
        z = jnp.einsum("bhsd->bhd", pk)
        num = jnp.einsum("bhqd,bhde->bhqe", pq, kv)
        den = jnp.einsum("bhqd,bhd->bhq", pq, z)[..., None] + 1e-6
        o = num / den
        return (lambda x, *d: x.transpose(*d))(o, 0, 2, 1, 3).reshape(B, S, D) @ wo

    def _B_ref(x, w1, w2, w3, w4):
        B, S, D = x.shape
        h = _gelu(_layernorm(x, axis=-1) @ w1)
        c = D // 4
        g0 = jnp.pad(h[:, :, 0*c:1*c], ((0, 0), (1, 0), (0, 0)))[:, :S, :]
        g1 = jnp.pad(h[:, :, 1*c:2*c], ((0, 0), (0, 1), (0, 0)))[:, 1:, :]
        g2 = jnp.pad(h[:, :, 2*c:3*c], ((0, 0), (2, 0), (0, 0)))[:, :S, :]
        g3 = jnp.pad(h[:, :, 3*c:   ], ((0, 0), (0, 2), (0, 0)))[:, 2:, :]
        hs = jnp.concatenate([g0, g1, g2, g3], axis=-1) @ w2
        x1 = x + hs
        h2 = _gelu(_layernorm(x1, axis=-1) @ w3) @ w4
        return x1 + h2

    x = A_x
    g = _sigmoid((x * gate_w).sum(-1, keepdims=True))
    a = _A_ref(x, A_wqkv, A_wo)
    b = _B_ref(x, B_w1, B_w2, B_w3, B_w4)
    return g * a + (1 - g) * b
```

```python
import functools
import jax
import jax.numpy as jnp
from jax import lax
from jax.experimental import pallas as pl
from jax.experimental.pallas import tpu as pltpu

F32 = jnp.float32
BF16 = jnp.bfloat16

S, D, FF = 2048, 640, 1728
H, DH = 32, 20
NT = D // 128
HALO = 8
KV_ROWS = ((0, 144), (120, 264), (240, 400), (376, 520), (496, 640))
PADROWS = 672


def _gelu(x):
    c0 = 0.7978845608028654
    c1 = 0.7978845608028654 * 0.044715
    u = x * (c0 + c1 * (x * x))
    hx = 0.5 * x
    return hx + hx * jnp.tanh(u)


def _phi(t):
    return jnp.where(t > 0, t + 1.0, jnp.exp(t)) + 1e-6


def _ln(x):
    m = jnp.mean(x, axis=-1, keepdims=True)
    xc = x - m
    v = jnp.mean(xc * xc, axis=-1, keepdims=True)
    return xc * lax.rsqrt(v + 1e-5)


def _dot(a, b):
    return jnp.dot(a, b, preferred_element_type=F32)


def _dot_nt(a, b):
    return lax.dot_general(a, b, (((1,), (1,)), ((), ())), preferred_element_type=F32)


def make_kernel(T1, T2):
    N1 = S // T1
    N2 = S // T2

    def kernel(ax_hbm, wqkv_hbm, wo_hbm, w1_hbm, w2_hbm, w3t_hbm, w4_hbm, gw_hbm,
               out_hbm,
               ax, wq, wk, wv, wo, w1, w2, w3t, w4, gw,
               h_scr, g_scr, z_scr, m_scr, mp, wqp, zrow, obuf,
               sem_w, sem_ax, sem_out):
        def cp(src, dst, sem):
            return pltpu.make_async_copy(src, dst, sem)

        c_w1 = cp(w1_hbm, w1, sem_w.at[0])
        c_wk = cp(wqkv_hbm.at[:, pl.ds(D, D)], wk, sem_w.at[1])
        c_wv = cp(wqkv_hbm.at[:, pl.ds(2 * D, D)], wv, sem_w.at[2])
        c_wq = cp(wqkv_hbm.at[:, pl.ds(0, D)], wq, sem_w.at[3])
        c_wo = cp(wo_hbm, wo, sem_w.at[4])
        c_w2 = cp(w2_hbm, w2, sem_w.at[5])
        c_w3 = cp(w3t_hbm, w3t, sem_w.at[6])
        c_w4 = cp(w4_hbm, w4, sem_w.at[7])
        c_gw = cp(gw_hbm, gw, sem_w.at[8])

        def c_ax(i):
            return cp(ax_hbm.at[0, pl.ds(i * T1, T1), :], ax.at[pl.ds(i * T1, T1), :], sem_ax.at[i])

        c_ax(0).start()
        c_w1.start()
        c_wk.start()
        for i in range(1, N1):
            c_ax(i).start()
        c_wq.start()
        c_wv.start()
        c_wo.start()
        c_gw.start()
        c_w2.start()
        c_w3.start()
        c_w4.start()

        zeros8 = jnp.zeros((HALO, 128), F32)
        for j in range(NT):
            h_scr[j, 0:HALO, :] = zeros8
            h_scr[j, HALO + S:HALO + S + HALO, :] = zeros8
        g_scr[...] = jnp.zeros((D, D), F32)
        z_scr[...] = jnp.zeros((PADROWS, 128), F32)

        c_w1.wait()

        def phase1(i, carry):
            r0 = pl.multiple_of(i * T1, T1)
            c_ax(i).wait()
            xa = ax[pl.ds(r0, T1), :]
            h = _gelu(_dot(_ln(xa.astype(F32)).astype(BF16), w1[...]))
            for j in range(NT):
                h_scr[j, pl.ds(r0 + HALO, T1), :] = h[:, 128 * j:128 * (j + 1)]

            @pl.when(i == 0)
            def _():
                c_wk.wait()

            xa = ax[pl.ds(r0, T1), :]
            pkT = _phi(_dot(xa, wk[...])).T
            acc = pkT[:, 0:128]
            for t in range(1, T1 // 128):
                acc = acc + pkT[:, 128 * t:128 * (t + 1)]
            z_scr[0:D, :] += acc
            g_scr[...] += _dot(pkT.astype(BF16), xa)
            return carry

        lax.fori_loop(0, N1, phase1, 0)

        c_wq.wait()
        c_wv.wait()
        c_wo.wait()
        c_gw.wait()
        c_w2.wait()
        c_w3.wait()
        c_w4.wait()

        wqT = wq[...].astype(F32).T
        for n in range(NT):
            m_scr[n, 0:D, :] = wqT[:, 128 * n:128 * (n + 1)]
        for d in range(DH):
            for n in range(NT):
                wqp[32 * d:32 * (d + 1), 128 * n:128 * (n + 1)] = (
                    m_scr[n, pl.ds(d, H, stride=DH), :].astype(BF16))

        for n in range(NT):
            m_scr[n, 0:D, :] = jnp.zeros((D, 128), F32)
        for j, (lo, hi) in enumerate(KV_ROWS):
            gj = g_scr[lo:hi, :].astype(BF16)
            kv = _dot(gj, wv[:, 128 * j:128 * (j + 1)])
            rh = (lax.broadcasted_iota(jnp.int32, (hi - lo, 128), 0) + lo) // DH
            ch = (lax.broadcasted_iota(jnp.int32, (hi - lo, 128), 1) + 128 * j) // DH
            kv = jnp.where(rh == ch, kv, 0.0).astype(BF16)
            mj = _dot(kv, wo[128 * j:128 * (j + 1), :])
            for n in range(NT):
                m_scr[n, lo:hi, :] += mj[:, 128 * n:128 * (n + 1)]
        for d in range(DH):
            for n in range(NT):
                mp[32 * d:32 * (d + 1), 128 * n:128 * (n + 1)] = (
                    m_scr[n, pl.ds(d, H, stride=DH), :].astype(BF16))
        zp = jnp.concatenate([z_scr[pl.ds(d, H, stride=DH), :] for d in range(DH)], axis=0)
        zrow[...] = jnp.sum(zp.T, axis=0, keepdims=True)

        lane = lax.broadcasted_iota(jnp.int32, (T2, 128), 1)

        def c_out(i, slot):
            return cp(obuf.at[slot], out_hbm.at[0, pl.ds(i * T2, T2), :], sem_out.at[slot])

        def phase2(i, carry):
            r0 = pl.multiple_of(i * T2, T2)
            slot = i % 2

            def hrow(j, off):
                return h_scr[j, pl.ds(r0 + HALO + off, T2), :]

            hs = jnp.concatenate([
                hrow(0, -1),
                jnp.where(lane < 32, hrow(1, -1), hrow(1, 1)),
                jnp.where(lane < 64, hrow(2, 1), hrow(2, -2)),
                jnp.where(lane < 96, hrow(3, -2), hrow(3, 2)),
                hrow(4, 2),
            ], axis=1).astype(BF16)
            xa = ax[pl.ds(r0, T2), :]
            xf = xa.astype(F32)
            x1 = xf + _dot(hs, w2[...])
            u = _gelu(_dot_nt(_ln(x1).astype(BF16), w3t[...])).astype(BF16)
            b = x1 + _dot(u, w4[...])

            pq = _phi(_dot_nt(xa, wqp[...]))
            z = zrow[...]
            pz = pq * z
            den = pz[:, 0:128]
            for t in range(1, NT):
                den = den + pz[:, 128 * t:128 * (t + 1)]
            den = den + pltpu.roll(den, 64, 1)
            den = den + pltpu.roll(den, 32, 1)
            g = jax.nn.sigmoid(jnp.sum(xf * gw[...].astype(F32), axis=-1, keepdims=True))
            r = g / (den + 1e-6)
            pqn = jnp.concatenate([pq[:, 128 * t:128 * (t + 1)] * r for t in range(NT)], axis=1).astype(BF16)
            a = _dot(pqn, mp[...])
            res = (a + (1.0 - g) * b).astype(BF16)

            @pl.when(i >= 2)
            def _():
                c_out(i - 2, slot).wait()

            obuf[slot] = res
            c_out(i, slot).start()
            return carry

        lax.fori_loop(0, N2, phase2, 0)
        for i in range(max(N2 - 2, 0), N2):
            c_out(i, i % 2).wait()

    scratch = [
        pltpu.VMEM((S, D), BF16),
        pltpu.VMEM((D, D), BF16),
        pltpu.VMEM((D, D), BF16),
        pltpu.VMEM((D, D), BF16),
        pltpu.VMEM((D, D), BF16),
        pltpu.VMEM((D, D), BF16),
        pltpu.VMEM((D, D), BF16),
        pltpu.VMEM((FF, D), BF16),
        pltpu.VMEM((FF, D), BF16),
        pltpu.VMEM((1, D), BF16),
        pltpu.VMEM((NT, S + 2 * HALO, 128), F32),
        pltpu.VMEM((D, D), F32),
        pltpu.VMEM((PADROWS, 128), F32),
        pltpu.VMEM((NT, PADROWS, 128), F32),
        pltpu.VMEM((D, D), BF16),
        pltpu.VMEM((D, D), BF16),
        pltpu.VMEM((1, D), F32),
        pltpu.VMEM((2, T2, D), BF16),
        pltpu.SemaphoreType.DMA((9,)),
        pltpu.SemaphoreType.DMA((N1,)),
        pltpu.SemaphoreType.DMA((2,)),
    ]
    return kernel, scratch


_KERNEL, _SCRATCH = make_kernel(512, 512)


@jax.jit
def pallas_gated_mix__linear_attn_block__mixer_s_mlp__prompt_kernel(
    A_x: jax.Array,
    A_wqkv: jax.Array,
    A_wo: jax.Array,
    B_x: jax.Array,
    B_w1: jax.Array,
    B_w2: jax.Array,
    B_w3: jax.Array,
    B_w4: jax.Array,
    gate_w: jax.Array,
):
    del B_x
    return pl.pallas_call(
        _KERNEL,
        out_shape=jax.ShapeDtypeStruct((1, S, D), BF16),
        in_specs=[pl.BlockSpec(memory_space=pl.ANY)] * 8,
        out_specs=pl.BlockSpec(memory_space=pl.ANY),
        scratch_shapes=_SCRATCH,
        compiler_params=pltpu.CompilerParams(vmem_limit_bytes=100 * 2**20),
    )(A_x, A_wqkv, A_wo, B_w1, B_w2, B_w3.T, B_w4, gate_w.reshape(1, D))
```

```python
import functools
import jax
import jax.numpy as jnp
from jax import lax
from jax.experimental import pallas as pl
from jax.experimental.pallas import tpu as pltpu

F32 = jnp.float32
BF16 = jnp.bfloat16

S, D, FF = 2048, 640, 1728
H, DH = 32, 20
NT = D // 128
HALO = 8
KV_ROWS = ((0, 144), (120, 264), (240, 400), (376, 520), (496, 640))
PADROWS = 672
R1 = 512


def _gelu(x):
    c0 = 0.7978845608028654
    c1 = 0.7978845608028654 * 0.044715
    u = x * (c0 + c1 * (x * x))
    hx = 0.5 * x
    return hx + hx * jnp.tanh(u)


def _phi(t):
    return jnp.where(t > 0, t + 1.0, jnp.exp(t)) + 1e-6


def _ln(x):
    m = jnp.mean(x, axis=-1, keepdims=True)
    xc = x - m
    v = jnp.mean(xc * xc, axis=-1, keepdims=True)
    return xc * lax.rsqrt(v + 1e-5)


def _dot(a, b):
    return jnp.dot(a, b, preferred_element_type=F32)


def _dot_nt(a, b):
    return lax.dot_general(a, b, (((1,), (1,)), ((), ())), preferred_element_type=F32)


class _Scope:
    def __init__(self, on):
        self.on = on
        self.cur = None

    def exit(self):
        if self.cur is not None:
            self.cur.__exit__(None, None, None)
            self.cur = None

    def enter(self, name):
        self.exit()
        if self.on:
            self.cur = jax.named_scope(name)
            self.cur.__enter__()


def _al(x, m):
    return x if isinstance(x, int) else pl.multiple_of(x, m)


def make_kernel(T1=128, T2=128, U2=4, FT=True, WKS=384, SC=False):
    N1 = S // R1
    NS1 = R1 // T1
    N2 = S // T2
    XC = 256
    NXC = S // XC

    def kernel(ax_hbm, wqkv_hbm, wo_hbm, w1_hbm, w2_hbm, w3t_hbm, w4_hbm, gw_hbm,
               out_hbm,
               ax, wq, wk, wv, wo, w1, w2, w3t, w4, gw, gwf,
               h_scr, g_scr, z_scr, m_scr, t_scr, mp, wqp, zrow, pkt, obuf,
               sem_w, sem_wk, sem_ax, sem_out):
        def cp(src, dst, sem):
            return pltpu.make_async_copy(src, dst, sem)

        c_w1 = cp(w1_hbm, w1, sem_w.at[0])
        c_wv = cp(wqkv_hbm.at[:, pl.ds(2 * D, D)], wv, sem_w.at[2])
        c_wq = cp(wqkv_hbm.at[:, pl.ds(0, D)], wq, sem_w.at[3])
        c_wo = cp(wo_hbm, wo, sem_w.at[4])
        c_w2 = cp(w2_hbm, w2, sem_w.at[5])
        c_w3 = cp(w3t_hbm, w3t, sem_w.at[6])
        c_w4 = cp(w4_hbm, w4, sem_w.at[7])
        c_gw = cp(gw_hbm, gw, sem_w.at[8])

        wk_pieces = ((0, WKS), (WKS, D)) if WKS else ((0, D),)

        def c_wk(j):
            lo, hi = wk_pieces[j]
            return cp(wqkv_hbm.at[:, pl.ds(D + lo, hi - lo)], wk.at[:, pl.ds(lo, hi - lo)], sem_wk.at[j])

        def c_ax(i):
            return cp(ax_hbm.at[0, pl.ds(i * XC, XC), :], ax.at[pl.ds(i * XC, XC), :], sem_ax.at[i])

        c_ax(0).start()
        for j in range(len(wk_pieces)):
            c_wk(j).start()
        c_ax(1).start()

        def start_rest():
            c_ax(2).start(priority=1)
            c_ax(3).start(priority=1)
            c_w1.start(priority=1)
            for i in range(4, NXC):
                c_ax(i).start(priority=1)
            c_wq.start(priority=1)
            c_wv.start(priority=1)
            c_wo.start(priority=1)
            c_gw.start(priority=1)
            c_w2.start(priority=1)
            c_w3.start(priority=1)
            c_w4.start(priority=1)

        zeros8 = jnp.zeros((HALO, 128), F32)
        for j in range(NT):
            h_scr[j, 0:HALO, :] = zeros8
            h_scr[j, HALO + S:HALO + S + HALO, :] = zeros8
        z_scr[...] = jnp.zeros((PADROWS, 128), F32)

        def k_post(k, c0, first=False):
            rows = k.shape[0]
            pkT = _phi(k).T
            acc = pkT[:, 0:128]
            for t in range(1, rows // 128):
                acc = acc + pkT[:, 128 * t:128 * (t + 1)]
            z_scr[0:D, :] += acc
            pkt[:, c0:c0 + rows] = pkT.astype(BF16)

        def b1_sub(r0):
            xs = ax[pl.ds(r0, T1), :]
            return _dot(_ln(xs.astype(F32)).astype(BF16), w1[...])

        def b1_post(hpre, r0):
            h = _gelu(hpre)
            for j in range(NT):
                h_scr[j, pl.ds(r0 + HALO, T1), :] = h[:, 128 * j:128 * (j + 1)]

        scope = _Scope(SC)
        scope.enter('pro_wait')
        c_ax(0).wait()
        c_wk(0).wait()
        start_rest()
        scope.enter('pro')
        xa0 = ax[0:XC, :]
        if WKS:
            k0a = _dot(xa0, wk[:, 0:WKS])
            c_wk(1).wait()
            k0b = _dot(xa0, wk[:, WKS:D])
            k0 = jnp.concatenate([k0a, k0b], axis=1)
        else:
            k0 = _dot(xa0, wk[...])
        c_ax(1).wait()
        xb0 = ax[XC:2 * XC, :]
        k1 = _dot(xb0, wk[...])
        k_post(k0, 0)
        g_scr[...] = _dot(pkt[:, 0:XC], xa0)
        k_post(k1, XC)
        g_scr[...] += _dot(pkt[:, XC:2 * XC], xb0)
        c_w1.wait()

        def phase1(i, carry):
            r0 = _al(i * R1, R1)
            rb = _al((i - 1) * R1, R1)
            c_ax(2 * i).wait()
            c_ax(2 * i + 1).wait()
            for s in range(NS1):
                xs = ax[pl.ds(r0 + s * T1, T1), :]
                k = _dot(xs, wk[...])
                hpre = b1_sub(rb + s * T1)
                k_post(k, s * T1)
                b1_post(hpre, rb + s * T1)
            g_scr[...] += _dot(pkt[...], ax[pl.ds(r0, R1), :])
            return carry

        scope.enter('p1')
        lax.fori_loop(1, N1, phase1, 0)
        scope.enter('epi')

        c_wq.wait()
        c_wv.wait()
        c_wo.wait()
        c_gw.wait()
        c_w2.wait()
        c_w3.wait()
        c_w4.wait()

        rb = (N1 - 1) * R1
        for n in range(NT):
            m_scr[n, 0:D, :] = jnp.zeros((D, 128), F32)
        kvs = []
        for j, (lo, hi) in enumerate(KV_ROWS):
            gj = g_scr[lo:hi, :].astype(BF16)
            kvs.append(_dot(gj, wv[:, 128 * j:128 * (j + 1)]))
        hpre = b1_sub(rb)
        for j in range(NT):
            wqT = wq[:, 128 * j:128 * (j + 1)].astype(F32).T
            for n in range(NT):
                t_scr[n, 128 * j:128 * (j + 1), :] = wqT[:, 128 * n:128 * (n + 1)]
        for j, (lo, hi) in enumerate(KV_ROWS):
            rh = (lax.broadcasted_iota(jnp.int32, (hi - lo, 128), 0) + lo) // DH
            ch = (lax.broadcasted_iota(jnp.int32, (hi - lo, 128), 1) + 128 * j) // DH
            kv = jnp.where(rh == ch, kvs[j], 0.0).astype(BF16)
            mj = _dot(kv, wo[128 * j:128 * (j + 1), :])
            for n in range(NT):
                m_scr[n, lo:hi, :] += mj[:, 128 * n:128 * (n + 1)]

        def gather_wq():
            for d in range(DH):
                for n in range(NT):
                    wqp[32 * d:32 * (d + 1), 128 * n:128 * (n + 1)] = (
                        t_scr[n, pl.ds(d, H, stride=DH), :].astype(BF16))

        def gather_m():
            for d in range(DH):
                for n in range(NT):
                    mp[32 * d:32 * (d + 1), 128 * n:128 * (n + 1)] = (
                        m_scr[n, pl.ds(d, H, stride=DH), :].astype(BF16))

        def gather_z():
            gwf[...] = gw[...].astype(F32).reshape(1, D)
            zp = jnp.concatenate([z_scr[pl.ds(d, H, stride=DH), :] for d in range(DH)], axis=0)
            zrow[...] = jnp.sum(zp.T, axis=0, keepdims=True)

        extra = [gather_wq, gather_m, gather_z]
        for s in range(NS1):
            nxt = b1_sub(rb + (s + 1) * T1) if s + 1 < NS1 else None
            b1_post(hpre, rb + s * T1)
            if extra:
                extra.pop(0)()
            hpre = nxt
        for e in extra:
            e()

        lane = lax.broadcasted_iota(jnp.int32, (T2, 128), 1)

        def c_out(i):
            return cp(obuf.at[pl.ds(i * T2, T2), :], out_hbm.at[0, pl.ds(i * T2, T2), :], sem_out.at[i])

        def phase2(i):
            r0 = _al(i * T2, T2)

            def hrow(j, off):
                return h_scr[j, pl.ds(r0 + HALO + off, T2), :]

            xa = ax[pl.ds(r0, T2), :]
            q = _dot_nt(xa, wqp[...])
            hs = jnp.concatenate([
                hrow(0, -1),
                jnp.where(lane < 32, hrow(1, -1), hrow(1, 1)),
                jnp.where(lane < 64, hrow(2, 1), hrow(2, -2)),
                jnp.where(lane < 96, hrow(3, -2), hrow(3, 2)),
                hrow(4, 2),
            ], axis=1).astype(BF16)
            xf = xa.astype(F32)
            x1 = xf + _dot(hs, w2[...])

            pq = _phi(q)
            z = zrow[...]
            pz = pq * z
            den = pz[:, 0:128]
            for t in range(1, NT):
                den = den + pz[:, 128 * t:128 * (t + 1)]
            den = den + pltpu.roll(den, 64, 1)
            den = den + pltpu.roll(den, 32, 1)
            g = jax.nn.sigmoid(jnp.sum(xf * gwf[...], axis=-1, keepdims=True))
            r = g / (den + 1e-6)
            pqn = jnp.concatenate([pq[:, 128 * t:128 * (t + 1)] * r for t in range(NT)], axis=1).astype(BF16)
            a = _dot(pqn, mp[...])
            ln2 = _ln(x1).astype(BF16)
            omg = 1.0 - g
            base = a + omg * x1
            if FT:
                FM = 1664
                u_main = _gelu(_dot_nt(ln2, w3t[0:FM, :])).astype(BF16)
                u_last = _gelu(_dot_nt(w3t[FM:FF, :], ln2)).T.astype(BF16)
                u = jnp.concatenate([u_main, u_last], axis=1)
            else:
                u = _gelu(_dot_nt(ln2, w3t[...])).astype(BF16)
            res = (base + omg * _dot(u, w4[...])).astype(BF16)
            obuf[pl.ds(r0, T2), :] = res
            c_out(i).start()

        def body2(ii, c):
            for u in range(U2):
                phase2(ii * U2 + u)
            return c
        scope.enter('p2')
        lax.fori_loop(0, N2 // U2, body2, 0)
        scope.enter('tail')
        for i in range(N2):
            c_out(i).wait()
        scope.exit()

    scratch = [
        pltpu.VMEM((S, D), BF16),
        pltpu.VMEM((D, D), BF16),
        pltpu.VMEM((D, D), BF16),
        pltpu.VMEM((D, D), BF16),
        pltpu.VMEM((D, D), BF16),
        pltpu.VMEM((D, D), BF16),
        pltpu.VMEM((D, D), BF16),
        pltpu.VMEM((FF, D), BF16),
        pltpu.VMEM((FF, D), BF16),
        pltpu.VMEM((D,), BF16),
        pltpu.VMEM((1, D), F32),
        pltpu.VMEM((NT, S + 2 * HALO, 128), F32),
        pltpu.VMEM((D, D), F32),
        pltpu.VMEM((PADROWS, 128), F32),
        pltpu.VMEM((NT, PADROWS, 128), F32),
        pltpu.VMEM((NT, PADROWS, 128), F32),
        pltpu.VMEM((D, D), BF16),
        pltpu.VMEM((D, D), BF16),
        pltpu.VMEM((1, D), F32),
        pltpu.VMEM((D, R1), BF16),
        pltpu.VMEM((S, D), BF16),
        pltpu.SemaphoreType.DMA((9,)),
        pltpu.SemaphoreType.DMA((2,)),
        pltpu.SemaphoreType.DMA((NXC,)),
        pltpu.SemaphoreType.DMA((N2,)),
    ]
    return kernel, scratch


_KERNEL, _SCRATCH = make_kernel(FT=True, WKS=256)


@jax.jit
def pallas_gated_mix__linear_attn_block__mixer_s_mlp__prompt_kernel(
    A_x: jax.Array,
    A_wqkv: jax.Array,
    A_wo: jax.Array,
    B_x: jax.Array,
    B_w1: jax.Array,
    B_w2: jax.Array,
    B_w3: jax.Array,
    B_w4: jax.Array,
    gate_w: jax.Array,
):
    del B_x
    return pl.pallas_call(
        _KERNEL,
        out_shape=jax.ShapeDtypeStruct((1, S, D), BF16),
        in_specs=[pl.BlockSpec(memory_space=pl.ANY)] * 8,
        out_specs=pl.BlockSpec(memory_space=pl.ANY),
        scratch_shapes=_SCRATCH,
        compiler_params=pltpu.CompilerParams(vmem_limit_bytes=100 * 2**20),
    )(A_x, A_wqkv, A_wo, B_w1, B_w2, B_w3.T, B_w4, gate_w)
```

```python
import jax
import jax.numpy as jnp
from jax import lax
from jax.experimental import pallas as pl
from jax.experimental.pallas import tpu as pltpu

F32 = jnp.float32
BF16 = jnp.bfloat16

S, D, FF = 2048, 640, 1728
H, DH = 32, 20
NT = D // 128
HALO = 8
KV_ROWS = ((0, 144), (120, 264), (240, 400), (376, 520), (496, 640))
PADROWS = 672
R1 = 512
XC = 256
NXC = S // XC
FM = 1664


def _gelu(x):
    c0 = 0.7978845608028654
    c1 = 0.7978845608028654 * 0.044715
    u = x * (c0 + c1 * (x * x))
    hx = 0.5 * x
    return hx + hx * jnp.tanh(u)


def _phi(t):
    return jnp.where(t > 0, t + 1.0, jnp.exp(t)) + 1e-6


def _ln(x):
    m = jnp.mean(x, axis=-1, keepdims=True)
    xc = x - m
    v = jnp.mean(xc * xc, axis=-1, keepdims=True)
    return xc * lax.rsqrt(v + 1e-5)


def _dot(a, b):
    return jnp.dot(a, b, preferred_element_type=F32)


def _dot_nt(a, b):
    return lax.dot_general(a, b, (((1,), (1,)), ((), ())), preferred_element_type=F32)


class _Scope:
    def __init__(self, on):
        self.on = on
        self.cur = None

    def exit(self):
        if self.cur is not None:
            self.cur.__exit__(None, None, None)
            self.cur = None

    def enter(self, name):
        self.exit()
        if self.on:
            self.cur = jax.named_scope(name)
            self.cur.__enter__()


def _al(x, m):
    return x if isinstance(x, int) else pl.multiple_of(x, m)


def make_kernel(T1=128, T2=128, U2=4, WKS=256, SC=False, GP1=False, MNOZ=True, EORD=0, SPL=True, WQP1=True):
    N1 = S // R1
    NS1 = R1 // T1
    N2 = S // T2

    def kernel(ax_hbm, wqkv_hbm, wo_hbm, w1_hbm, w2_hbm, w3t_hbm, w4_hbm, gw_hbm,
               out_hbm,
               ax, wq, wk, wv, wo, w1, w2, w3t, w4, gw, gwf,
               h_scr, g_scr, z_scr, m_scr, t_scr, mp, wqp, zrow, pkt, gate, obuf,
               sem_w, sem_wk, sem_wq, sem_ax, sem_out):
        def cp(src, dst, sem):
            return pltpu.make_async_copy(src, dst, sem)

        c_w1 = cp(w1_hbm, w1, sem_w.at[0])
        c_gw = cp(gw_hbm, gw, sem_w.at[1])
        c_wv = cp(wqkv_hbm.at[:, pl.ds(2 * D, D)], wv, sem_w.at[2])
        c_wo = cp(wo_hbm, wo, sem_w.at[4])
        c_w2 = cp(w2_hbm, w2, sem_w.at[5])
        c_w3 = cp(w3t_hbm, w3t, sem_w.at[6])
        c_w4 = cp(w4_hbm, w4, sem_w.at[7])

        wk_pieces = ((0, WKS), (WKS, D))

        def c_wq(j):
            src_j = j if not isinstance(j, int) else min(j, NT - 1)
            src_j = jnp.minimum(j, NT - 1) if not isinstance(j, int) else src_j
            return cp(wqkv_hbm.at[:, pl.ds(_al(128 * src_j, 128), 128)], wq.at[j], sem_wq.at[j])

        def c_wk(j):
            lo, hi = wk_pieces[j]
            return cp(wqkv_hbm.at[:, pl.ds(D + lo, hi - lo)], wk.at[:, pl.ds(lo, hi - lo)], sem_wk.at[j])

        def c_ax(i):
            return cp(ax_hbm.at[0, pl.ds(i * XC, XC), :], ax.at[pl.ds(i * XC, XC), :], sem_ax.at[i])

        c_ax(0).start()
        c_wk(0).start()
        c_wk(1).start()
        c_ax(1).start()

        def start_a():
            c_w1.start()
            c_ax(2).start()
            c_ax(3).start()
            c_gw.start()

        def start_b():
            if WQP1:
                c_wq(0).start()
                c_wq(1).start()
            c_ax(4).start()
            c_ax(5).start()

        def start_c():
            if WQP1:
                c_wq(2).start()
                c_wq(3).start()
            c_ax(6).start()
            c_ax(7).start()
            if WQP1:
                c_wq(4).start()
                c_wq(5).start()
            else:
                for j in range(NT):
                    c_wq(j).start(priority=1)
            c_wv.start(priority=1)
            c_wo.start(priority=1)
            c_w2.start(priority=1)
            c_w3.start(priority=1)
            c_w4.start(priority=1)

        zeros8 = jnp.zeros((HALO, 128), F32)
        for j in range(NT):
            h_scr[j, 0:HALO, :] = zeros8
            h_scr[j, HALO + S:HALO + S + HALO, :] = zeros8
        z_scr[...] = jnp.zeros((PADROWS, 128), F32)

        def k_post(k, c0):
            rows = k.shape[0]
            pkT = _phi(k).T
            acc = pkT[:, 0:128]
            for t in range(1, rows // 128):
                acc = acc + pkT[:, 128 * t:128 * (t + 1)]
            z_scr[0:D, :] += acc
            pkt[:, c0:c0 + rows] = pkT.astype(BF16)

        def gate_of(xf):
            return jax.nn.sigmoid(jnp.sum(xf * gwf[...], axis=-1, keepdims=True))

        def b1_sub(r0):
            xf = ax[pl.ds(r0, T1), :].astype(F32)
            hpre = _dot(_ln(xf).astype(BF16), w1[...])
            if GP1:
                gate[pl.ds(r0, T1), :] = jnp.broadcast_to(gate_of(xf), (T1, 128))
            return hpre

        def b1_post(hpre, r0):
            h = _gelu(hpre)
            for j in range(NT):
                h_scr[j, pl.ds(r0 + HALO, T1), :] = h[:, 128 * j:128 * (j + 1)]

        scope = _Scope(SC)
        scope.enter('pro_wait')
        c_ax(0).wait()
        c_wk(0).wait()
        start_a()
        scope.enter('pro')
        def dot_rows(a, b, parts):
            if parts == 1:
                return _dot(a, b)
            n = a.shape[0] // parts
            return jnp.concatenate([_dot(a[p * n:(p + 1) * n, :], b) for p in range(parts)], axis=0)

        xa0 = ax[0:XC, :]
        k0a = dot_rows(xa0, wk[:, 0:WKS], 2 if SPL else 1)
        c_wk(1).wait()
        start_b()
        k0b = dot_rows(xa0, wk[:, WKS:D], 4 if SPL else 1)
        k0 = jnp.concatenate([k0a, k0b], axis=1)
        c_ax(1).wait()
        start_c()
        xb0 = ax[XC:2 * XC, :]
        k1 = _dot(xb0, wk[...])
        k_post(k0, 0)
        g_scr[...] = _dot(pkt[:, 0:XC], xa0)
        k_post(k1, XC)
        if SPL:
            for p in range(2):
                g_scr[320 * p:320 * (p + 1), :] += _dot(pkt[320 * p:320 * (p + 1), XC:2 * XC], xb0)
        else:
            g_scr[...] += _dot(pkt[:, XC:2 * XC], xb0)
        c_w1.wait()
        c_gw.wait()
        gwf[...] = gw[...].astype(F32).reshape(1, D)

        def wq_t_chunk(j):
            wqT = wq[j].astype(F32).T
            for n in range(NT):
                t_scr[n, pl.ds(_al(128 * j, 128), 128), :] = wqT[:, 128 * n:128 * (n + 1)]


        def phase1(i, carry):
            r0 = _al(i * R1, R1)
            rb = _al((i - 1) * R1, R1)
            c_ax(2 * i).wait()
            c_ax(2 * i + 1).wait()
            if WQP1:
                c_wq(2 * i - 2).wait()
                c_wq(2 * i - 1).wait()
            for s in range(NS1):
                xs = ax[pl.ds(r0 + s * T1, T1), :]
                k = _dot(xs, wk[...])
                hpre = b1_sub(rb + s * T1)
                k_post(k, s * T1)
                b1_post(hpre, rb + s * T1)
                if WQP1 and s < 2:
                    wq_t_chunk(2 * (i - 1) + s)
            g_scr[...] += _dot(pkt[...], ax[pl.ds(r0, R1), :])
            return carry

        scope.enter('p1')
        lax.fori_loop(1, N1, phase1, 0)
        scope.enter('epi')

        if not WQP1:
            for j in range(NT):
                c_wq(j).wait()
        c_wv.wait()
        c_wo.wait()
        c_w2.wait()
        c_w3.wait()
        c_w4.wait()

        rb = (N1 - 1) * R1
        if not MNOZ:
            for n in range(NT):
                m_scr[n, 0:D, :] = jnp.zeros((D, 128), F32)
        kvs = []
        for j, (lo, hi) in enumerate(KV_ROWS):
            gj = g_scr[lo:hi, :].astype(BF16)
            kvs.append(_dot(gj, wv[:, 128 * j:128 * (j + 1)]))
        hpre = b1_sub(rb)

        def wq_t():
            if not WQP1:
                for j in range(NT):
                    wq_t_chunk(j)

        def m_build():
            prev = None
            for j, (lo, hi) in enumerate(KV_ROWS):
                rh = (lax.broadcasted_iota(jnp.int32, (hi - lo, 128), 0) + lo) // DH
                ch = (lax.broadcasted_iota(jnp.int32, (hi - lo, 128), 1) + 128 * j) // DH
                kv = jnp.where(rh == ch, kvs[j], 0.0).astype(BF16)
                mj = _dot(kv, wo[128 * j:128 * (j + 1), :])
                if MNOZ:
                    ov = 0 if prev is None else prev.shape[0]
                    nxt_lo = KV_ROWS[j + 1][0] if j + 1 < NT else hi
                    for n in range(NT):
                        col = mj[:, 128 * n:128 * (n + 1)]
                        if ov:
                            m_scr[n, lo:lo + ov, :] = col[0:ov] + prev[:, 128 * n:128 * (n + 1)]
                        m_scr[n, lo + ov:nxt_lo, :] = col[ov:nxt_lo - lo]
                    prev = mj[nxt_lo - lo:, :] if j + 1 < NT else None
                else:
                    for n in range(NT):
                        m_scr[n, lo:hi, :] += mj[:, 128 * n:128 * (n + 1)]

        def gather_wq():
            for d in range(DH):
                for n in range(NT):
                    wqp[32 * d:32 * (d + 1), 128 * n:128 * (n + 1)] = (
                        t_scr[n, pl.ds(d, H, stride=DH), :].astype(BF16))

        def gather_m():
            for d in range(DH):
                for n in range(NT):
                    mp[32 * d:32 * (d + 1), 128 * n:128 * (n + 1)] = (
                        m_scr[n, pl.ds(d, H, stride=DH), :].astype(BF16))

        def gather_z():
            zp = jnp.concatenate([z_scr[pl.ds(d, H, stride=DH), :] for d in range(DH)], axis=0)
            zrow[...] = jnp.sum(zp.T, axis=0, keepdims=True)

        if EORD == 0:
            wq_t()
            m_build()
            extra = [gather_wq, gather_m, gather_z]
        elif EORD == 1:
            m_build()
            wq_t()
            extra = [gather_m, gather_wq, gather_z]
        elif EORD == 2:
            gather_z()
            wq_t()
            m_build()
            extra = [gather_wq, gather_m]
        for s in range(NS1):
            nxt = b1_sub(rb + (s + 1) * T1) if s + 1 < NS1 else None
            b1_post(hpre, rb + s * T1)
            if extra:
                extra.pop(0)()
            hpre = nxt
        for e in extra:
            e()

        lane = lax.broadcasted_iota(jnp.int32, (T2, 128), 1)

        def c_out(i):
            return cp(obuf.at[pl.ds(i * T2, T2), :], out_hbm.at[0, pl.ds(i * T2, T2), :], sem_out.at[i])

        def st_q(i):
            r0 = _al(i * T2, T2)
            xa = ax[pl.ds(r0, T2), :]
            return _dot_nt(xa, wqp[...])

        def st_w2(i):
            r0 = _al(i * T2, T2)

            def hrow(j, off):
                return h_scr[j, pl.ds(r0 + HALO + off, T2), :]

            hs = jnp.concatenate([
                hrow(0, -1),
                jnp.where(lane < 32, hrow(1, -1), hrow(1, 1)),
                jnp.where(lane < 64, hrow(2, 1), hrow(2, -2)),
                jnp.where(lane < 96, hrow(3, -2), hrow(3, 2)),
                hrow(4, 2),
            ], axis=1).astype(BF16)
            return _dot(hs, w2[...])

        def st_phi(i, q):
            r0 = _al(i * T2, T2)
            pq = _phi(q)
            pz = pq * zrow[...]
            den = pz[:, 0:128]
            for t in range(1, NT):
                den = den + pz[:, 128 * t:128 * (t + 1)]
            den = den + pltpu.roll(den, 64, 1)
            den = den + pltpu.roll(den, 32, 1)
            if GP1:
                g = gate[pl.ds(r0, T2), :]
            else:
                g = gate_of(ax[pl.ds(r0, T2), :].astype(F32))
            r = g / (den + 1e-6)
            pqn = jnp.concatenate([pq[:, 128 * t:128 * (t + 1)] * r for t in range(NT)], axis=1).astype(BF16)
            return pqn, 1.0 - g

        def scale(v, omg):
            if GP1:
                return jnp.concatenate([v[:, 128 * t:128 * (t + 1)] * omg for t in range(NT)], axis=1)
            return v * omg

        def st_ln2(i, y):
            r0 = _al(i * T2, T2)
            x1 = ax[pl.ds(r0, T2), :].astype(F32) + y
            return x1, _ln(x1).astype(BF16)

        def st_w3(ln2):
            u_main = _gelu(_dot_nt(ln2, w3t[0:FM, :])).astype(BF16)
            u_last = _gelu(_dot_nt(w3t[FM:FF, :], ln2)).T.astype(BF16)
            return jnp.concatenate([u_main, u_last], axis=1)

        def st_fin(i, base, omg, h2):
            r0 = _al(i * T2, T2)
            obuf[pl.ds(r0, T2), :] = (base + scale(h2, omg)).astype(BF16)
            c_out(i).start()

        def run_tiles(i0, n):
            q = st_q(i0)
            y = st_w2(i0)
            pqn, omg = st_phi(i0, q)
            a = _dot(pqn, mp[...])
            x1, ln2 = st_ln2(i0, y)
            for u in range(n):
                i = i0 + u
                base = a + scale(x1, omg)
                omg_c = omg
                if u + 1 < n:
                    q = st_q(i + 1)
                uu = st_w3(ln2)
                if u + 1 < n:
                    y = st_w2(i + 1)
                    pqn, omg = st_phi(i + 1, q)
                h2 = _dot(uu, w4[...])
                if u + 1 < n:
                    x1, ln2 = st_ln2(i + 1, y)
                    a = _dot(pqn, mp[...])
                st_fin(i, base, omg_c, h2)

        def body2(ii, c):
            run_tiles(ii * U2, U2)
            return c

        scope.enter('p2')
        lax.fori_loop(0, N2 // U2, body2, 0)
        scope.enter('tail')
        for i in range(N2):
            c_out(i).wait()
        scope.exit()

    scratch = [
        pltpu.VMEM((S, D), BF16),
        pltpu.VMEM((NT + 1, D, 128), BF16),
        pltpu.VMEM((D, D), BF16),
        pltpu.VMEM((D, D), BF16),
        pltpu.VMEM((D, D), BF16),
        pltpu.VMEM((D, D), BF16),
        pltpu.VMEM((D, D), BF16),
        pltpu.VMEM((FF, D), BF16),
        pltpu.VMEM((FF, D), BF16),
        pltpu.VMEM((D,), BF16),
        pltpu.VMEM((1, D), F32),
        pltpu.VMEM((NT, S + 2 * HALO, 128), F32),
        pltpu.VMEM((D, D), F32),
        pltpu.VMEM((PADROWS, 128), F32),
        pltpu.VMEM((NT, PADROWS, 128), F32),
        pltpu.VMEM((NT, 768, 128), F32),
        pltpu.VMEM((D, D), BF16),
        pltpu.VMEM((D, D), BF16),
        pltpu.VMEM((1, D), F32),
        pltpu.VMEM((D, R1), BF16),
        pltpu.VMEM((S, 128), F32),
        pltpu.VMEM((S, D), BF16),
        pltpu.SemaphoreType.DMA((8,)),
        pltpu.SemaphoreType.DMA((2,)),
        pltpu.SemaphoreType.DMA((NT + 1,)),
        pltpu.SemaphoreType.DMA((NXC,)),
        pltpu.SemaphoreType.DMA((N2,)),
    ]
    return kernel, scratch


_KERNEL, _SCRATCH = make_kernel()


@jax.jit
def pallas_gated_mix__linear_attn_block__mixer_s_mlp__prompt_kernel(
    A_x: jax.Array,
    A_wqkv: jax.Array,
    A_wo: jax.Array,
    B_x: jax.Array,
    B_w1: jax.Array,
    B_w2: jax.Array,
    B_w3: jax.Array,
    B_w4: jax.Array,
    gate_w: jax.Array,
):
    del B_x
    return pl.pallas_call(
        _KERNEL,
        out_shape=jax.ShapeDtypeStruct((1, S, D), BF16),
        in_specs=[pl.BlockSpec(memory_space=pl.ANY)] * 8,
        out_specs=pl.BlockSpec(memory_space=pl.ANY),
        scratch_shapes=_SCRATCH,
        compiler_params=pltpu.CompilerParams(vmem_limit_bytes=100 * 2**20),
    )(A_x, A_wqkv, A_wo, B_w1, B_w2, B_w3.T, B_w4, gate_w)
```

```python
import jax
import jax.numpy as jnp
from jax import lax
from jax.experimental import pallas as pl
from jax.experimental.pallas import tpu as pltpu

F32 = jnp.float32
BF16 = jnp.bfloat16

S, D, FF = 2048, 640, 1728
H, DH = 32, 20
NT = D // 128
HALO = 8
KV_ROWS = ((0, 144), (120, 264), (240, 400), (376, 520), (496, 640))
PADROWS = 672
XC = 256
NXC = S // XC
R0 = 2 * XC
RL = 512
NL = (S - R0) // RL
CPT = RL // XC
WPT = (NT + 1) // NL
T1 = 128
NS1 = RL // T1
T2 = 128
U2 = 4
N2 = S // T2
FM = 1664
WK_PIECES = ((0, 256), (256, D))


def _gelu(x):
    c0 = 0.7978845608028654
    c1 = 0.7978845608028654 * 0.044715
    u = x * (c0 + c1 * (x * x))
    hx = 0.5 * x
    return hx + hx * jnp.tanh(u)


def _phi(t):
    return jnp.where(t > 0, t + 1.0, jnp.exp(t)) + 1e-6


def _ln(x):
    m = jnp.mean(x, axis=-1, keepdims=True)
    xc = x - m
    v = jnp.mean(xc * xc, axis=-1, keepdims=True)
    return xc * lax.rsqrt(v + 1e-5)


def _dot(a, b):
    return jnp.dot(a, b, preferred_element_type=F32)


def _dot_nt(a, b):
    return lax.dot_general(a, b, (((1,), (1,)), ((), ())), preferred_element_type=F32)


def _dot_rows(a, b, parts):
    n = a.shape[0] // parts
    return jnp.concatenate([_dot(a[p * n:(p + 1) * n, :], b) for p in range(parts)], axis=0)


def _al(x, m):
    return x if isinstance(x, int) else pl.multiple_of(x, m)


def _kernel(ax_hbm, wqkv_hbm, wo_hbm, w1_hbm, w2_hbm, w3t_hbm, w4_hbm, gw_hbm,
            out_hbm,
            ax, wq, wk, wv, wo, w1, w2, w3t, w4, gw, gwf,
            h_scr, g_scr, z_scr, m_scr, t_scr, mp, wqp, zrow, pkt, obuf,
            sem_w, sem_wk, sem_wq, sem_ax, sem_out):
    cp = pltpu.make_async_copy

    c_w1 = cp(w1_hbm, w1, sem_w.at[0])
    c_gw = cp(gw_hbm, gw, sem_w.at[1])
    late = (
        cp(wqkv_hbm.at[:, pl.ds(2 * D, D)], wv, sem_w.at[2]),
        cp(wo_hbm, wo, sem_w.at[3]),
        cp(w2_hbm, w2, sem_w.at[4]),
        cp(w3t_hbm, w3t, sem_w.at[5]),
        cp(w4_hbm, w4, sem_w.at[6]),
    )

    def c_wk(j):
        lo, hi = WK_PIECES[j]
        return cp(wqkv_hbm.at[:, pl.ds(D + lo, hi - lo)], wk.at[:, pl.ds(lo, hi - lo)], sem_wk.at[j])

    def c_wq(j):
        src = min(j, NT - 1) if isinstance(j, int) else jnp.minimum(j, NT - 1)
        return cp(wqkv_hbm.at[:, pl.ds(_al(128 * src, 128), 128)], wq.at[j], sem_wq.at[j])

    def c_ax(i):
        return cp(ax_hbm.at[0, pl.ds(i * XC, XC), :], ax.at[pl.ds(i * XC, XC), :], sem_ax.at[i])

    def c_out(i):
        return cp(obuf.at[pl.ds(i * T2, T2), :], out_hbm.at[0, pl.ds(i * T2, T2), :], sem_out.at[i])

    def start_trip(t):
        for c in range(CPT):
            c_ax(2 + t * CPT + c).start()
        for c in range(WPT):
            c_wq(t * WPT + c).start()

    c_ax(0).start()
    c_wk(0).start()
    c_wk(1).start()
    c_ax(1).start()

    zeros8 = jnp.zeros((HALO, 128), F32)
    for j in range(NT):
        h_scr[j, 0:HALO, :] = zeros8
        h_scr[j, HALO + S:HALO + S + HALO, :] = zeros8
    z_scr[...] = jnp.zeros((PADROWS, 128), F32)

    def k_post(k, c0):
        rows = k.shape[0]
        pkT = _phi(k).T
        acc = pkT[:, 0:128]
        for t in range(1, rows // 128):
            acc = acc + pkT[:, 128 * t:128 * (t + 1)]
        z_scr[0:D, :] += acc
        pkt[:, c0:c0 + rows] = pkT.astype(BF16)

    def mix_pre(r0):
        xf = ax[pl.ds(r0, T1), :].astype(F32)
        return _dot(_ln(xf).astype(BF16), w1[...])

    def mix_post(hpre, r0):
        h = _gelu(hpre)
        for j in range(NT):
            h_scr[j, pl.ds(r0 + HALO, T1), :] = h[:, 128 * j:128 * (j + 1)]

    def wq_t_chunk(j):
        wqT = wq[j].astype(F32).T
        for n in range(NT):
            t_scr[n, pl.ds(_al(128 * j, 128), 128), :] = wqT[:, 128 * n:128 * (n + 1)]

    c_ax(0).wait()
    c_wk(0).wait()
    c_w1.start()
    c_gw.start()
    xa0 = ax[0:XC, :]
    k0a = _dot_rows(xa0, wk[:, WK_PIECES[0][0]:WK_PIECES[0][1]], 2)
    c_wk(1).wait()
    start_trip(0)
    k0b = _dot_rows(xa0, wk[:, WK_PIECES[1][0]:WK_PIECES[1][1]], 4)
    k0 = jnp.concatenate([k0a, k0b], axis=1)
    c_ax(1).wait()
    for t in range(1, NL):
        start_trip(t)
    for c in late:
        c.start(priority=1)
    xb0 = ax[XC:2 * XC, :]
    k1 = _dot(xb0, wk[...])
    k_post(k0, 0)
    g_scr[...] = _dot(pkt[:, 0:XC], xa0)
    k_post(k1, XC)
    for p in range(2):
        g_scr[320 * p:320 * (p + 1), :] += _dot(pkt[320 * p:320 * (p + 1), XC:2 * XC], xb0)
    c_w1.wait()
    c_gw.wait()
    gwf[...] = gw[...].astype(F32).reshape(1, D)

    def phase1(t, carry):
        ra = _al(R0 + t * RL, XC)
        rb = _al(t * RL, XC)
        for c in range(CPT):
            c_ax(2 + t * CPT + c).wait()
        for c in range(WPT):
            c_wq(t * WPT + c).wait()
        for s in range(NS1):
            k = _dot(ax[pl.ds(ra + s * T1, T1), :], wk[...])
            hpre = mix_pre(rb + s * T1)
            k_post(k, s * T1)
            mix_post(hpre, rb + s * T1)
            if s < WPT:
                wq_t_chunk(t * WPT + s)
        g_scr[...] += _dot(pkt[...], ax[pl.ds(ra, RL), :])
        return carry

    lax.fori_loop(0, NL, phase1, 0)

    for c in late:
        c.wait()

    def m_build(kvs):
        prev = None
        for j, (lo, hi) in enumerate(KV_ROWS):
            rh = (lax.broadcasted_iota(jnp.int32, (hi - lo, 128), 0) + lo) // DH
            ch = (lax.broadcasted_iota(jnp.int32, (hi - lo, 128), 1) + 128 * j) // DH
            kv = jnp.where(rh == ch, kvs[j], 0.0).astype(BF16)
            mj = _dot(kv, wo[128 * j:128 * (j + 1), :])
            ov = 0 if prev is None else prev.shape[0]
            nxt = KV_ROWS[j + 1][0] if j + 1 < NT else hi
            for n in range(NT):
                col = mj[:, 128 * n:128 * (n + 1)]
                if ov:
                    m_scr[n, lo:lo + ov, :] = col[0:ov] + prev[:, 128 * n:128 * (n + 1)]
                m_scr[n, lo + ov:nxt, :] = col[ov:nxt - lo]
            prev = mj[nxt - lo:, :] if j + 1 < NT else None

    def gather(dst, src):
        for d in range(DH):
            for n in range(NT):
                dst[H * d:H * (d + 1), 128 * n:128 * (n + 1)] = (
                    src[n, pl.ds(d, H, stride=DH), :].astype(BF16))

    def gather_z():
        zp = jnp.concatenate([z_scr[pl.ds(d, H, stride=DH), :] for d in range(DH)], axis=0)
        zrow[...] = jnp.sum(zp.T, axis=0, keepdims=True)

    rb = S - R0
    kvs = [_dot(g_scr[lo:hi, :].astype(BF16), wv[:, 128 * j:128 * (j + 1)])
           for j, (lo, hi) in enumerate(KV_ROWS)]
    hpre = mix_pre(rb)
    m_build(kvs)
    extra = [lambda: gather(wqp, t_scr), lambda: gather(mp, m_scr), gather_z]
    for s in range(R0 // T1):
        nxt_pre = mix_pre(rb + (s + 1) * T1) if s + 1 < R0 // T1 else None
        mix_post(hpre, rb + s * T1)
        if s < len(extra):
            extra[s]()
        hpre = nxt_pre

    lane = lax.broadcasted_iota(jnp.int32, (T2, 128), 1)

    def st_q(i):
        return _dot_nt(ax[pl.ds(_al(i * T2, T2), T2), :], wqp[...])

    def st_w2(i):
        r0 = _al(i * T2, T2)

        def hrow(j, off):
            return h_scr[j, pl.ds(r0 + HALO + off, T2), :]

        hs = jnp.concatenate([
            hrow(0, -1),
            jnp.where(lane < 32, hrow(1, -1), hrow(1, 1)),
            jnp.where(lane < 64, hrow(2, 1), hrow(2, -2)),
            jnp.where(lane < 96, hrow(3, -2), hrow(3, 2)),
            hrow(4, 2),
        ], axis=1).astype(BF16)
        return _dot(hs, w2[...])

    def st_phi(i, q):
        pq = _phi(q)
        pz = pq * zrow[...]
        den = pz[:, 0:128]
        for t in range(1, NT):
            den = den + pz[:, 128 * t:128 * (t + 1)]
        den = den + pltpu.roll(den, 64, 1)
        den = den + pltpu.roll(den, 32, 1)
        xf = ax[pl.ds(_al(i * T2, T2), T2), :].astype(F32)
        g = jax.nn.sigmoid(jnp.sum(xf * gwf[...], axis=-1, keepdims=True))
        r = g / (den + 1e-6)
        pqn = jnp.concatenate([pq[:, 128 * t:128 * (t + 1)] * r for t in range(NT)], axis=1)
        return pqn.astype(BF16), 1.0 - g

    def st_ln2(i, y):
        x1 = ax[pl.ds(_al(i * T2, T2), T2), :].astype(F32) + y
        return x1, _ln(x1).astype(BF16)

    def st_w3(ln2):
        u_main = _gelu(_dot_nt(ln2, w3t[0:FM, :])).astype(BF16)
        u_last = _gelu(_dot_nt(w3t[FM:FF, :], ln2)).T.astype(BF16)
        return jnp.concatenate([u_main, u_last], axis=1)

    def phase2(trip, carry):
        i0 = trip * U2
        q = st_q(i0)
        y = st_w2(i0)
        pqn, omg = st_phi(i0, q)
        a = _dot(pqn, mp[...])
        x1, ln2 = st_ln2(i0, y)
        for u in range(U2):
            i = i0 + u
            more = u + 1 < U2
            if more:
                q = st_q(i + 1)
            base = a + omg * x1
            omg_i = omg
            uu = st_w3(ln2)
            if more:
                y = st_w2(i + 1)
                pqn, omg = st_phi(i + 1, q)
            h2 = _dot(uu, w4[...])
            if more:
                x1, ln2 = st_ln2(i + 1, y)
                a = _dot(pqn, mp[...])
            obuf[pl.ds(_al(i * T2, T2), T2), :] = (base + omg_i * h2).astype(BF16)
            c_out(i).start()
        return carry

    lax.fori_loop(0, N2 // U2, phase2, 0)
    for i in range(N2):
        c_out(i).wait()


_SCRATCH = [
    pltpu.VMEM((S, D), BF16),
    pltpu.VMEM((NT + 1, D, 128), BF16),
    pltpu.VMEM((D, D), BF16),
    pltpu.VMEM((D, D), BF16),
    pltpu.VMEM((D, D), BF16),
    pltpu.VMEM((D, D), BF16),
    pltpu.VMEM((D, D), BF16),
    pltpu.VMEM((FF, D), BF16),
    pltpu.VMEM((FF, D), BF16),
    pltpu.VMEM((D,), BF16),
    pltpu.VMEM((1, D), F32),
    pltpu.VMEM((NT, S + 2 * HALO, 128), F32),
    pltpu.VMEM((D, D), F32),
    pltpu.VMEM((PADROWS, 128), F32),
    pltpu.VMEM((NT, PADROWS, 128), F32),
    pltpu.VMEM((NT, 128 * (NT + 1), 128), F32),
    pltpu.VMEM((D, D), BF16),
    pltpu.VMEM((D, D), BF16),
    pltpu.VMEM((1, D), F32),
    pltpu.VMEM((D, RL), BF16),
    pltpu.VMEM((S, D), BF16),
    pltpu.SemaphoreType.DMA((7,)),
    pltpu.SemaphoreType.DMA((len(WK_PIECES),)),
    pltpu.SemaphoreType.DMA((NT + 1,)),
    pltpu.SemaphoreType.DMA((NXC,)),
    pltpu.SemaphoreType.DMA((N2,)),
]


@jax.jit
def pallas_gated_mix__linear_attn_block__mixer_s_mlp__prompt_kernel(
    A_x: jax.Array,
    A_wqkv: jax.Array,
    A_wo: jax.Array,
    B_x: jax.Array,
    B_w1: jax.Array,
    B_w2: jax.Array,
    B_w3: jax.Array,
    B_w4: jax.Array,
    gate_w: jax.Array,
):
    del B_x
    return pl.pallas_call(
        _kernel,
        out_shape=jax.ShapeDtypeStruct((1, S, D), BF16),
        in_specs=[pl.BlockSpec(memory_space=pl.ANY)] * 8,
        out_specs=pl.BlockSpec(memory_space=pl.ANY),
        scratch_shapes=_SCRATCH,
        compiler_params=pltpu.CompilerParams(vmem_limit_bytes=100 * 2**20),
    )(A_x, A_wqkv, A_wo, B_w1, B_w2, B_w3.T, B_w4, gate_w)
```

```python
import jax
import jax.numpy as jnp
from jax import lax
from jax.experimental import pallas as pl
from jax.experimental.pallas import tpu as pltpu

F32 = jnp.float32
BF16 = jnp.bfloat16

S, D, FF = 2048, 640, 1728
H, DH = 32, 20
NT = D // 128
HALO = 8
KV_ROWS = ((0, 144), (120, 264), (240, 400), (376, 520), (496, 640))
PADROWS = 672
XC = 256
NXC = S // XC
R0 = 2 * XC
RL = 512
NL = (S - R0) // RL
CPT = RL // XC
WPT = (NT + 1) // NL
T1 = 128
NS1 = RL // T1
T2 = 128
U2 = 4
N2 = S // T2
FM = 1664
WK_PIECES = ((0, 128), (128, 384), (384, D))


def _gelu(x):
    c0 = 0.7978845608028654
    c1 = 0.7978845608028654 * 0.044715
    u = x * (c0 + c1 * (x * x))
    hx = 0.5 * x
    return hx + hx * jnp.tanh(u)


def _phi(t):
    return jnp.where(t > 0, t + 1.0, jnp.exp(t)) + 1e-6


def _ln(x):
    m = jnp.mean(x, axis=-1, keepdims=True)
    xc = x - m
    v = jnp.mean(xc * xc, axis=-1, keepdims=True)
    return xc * lax.rsqrt(v + 1e-5)


def _dot(a, b):
    return jnp.dot(a, b, preferred_element_type=F32)


def _dot_nt(a, b):
    return lax.dot_general(a, b, (((1,), (1,)), ((), ())), preferred_element_type=F32)


def _dot_rows(a, b, parts):
    n = a.shape[0] // parts
    return jnp.concatenate([_dot(a[p * n:(p + 1) * n, :], b) for p in range(parts)], axis=0)


def _al(x, m):
    return x if isinstance(x, int) else pl.multiple_of(x, m)


def _kernel(ax_hbm, wqkv_hbm, wo_hbm, w1_hbm, w2_hbm, w3t_hbm, w4_hbm, gw_hbm,
            out_hbm,
            ax, wq, wk, wv, wo, w1, w2, w3t, w4, gw, gwf,
            h_scr, g_scr, z_scr, m_scr, t_scr, mp, wqp, zrow, pkt, obuf,
            sem_w, sem_wk, sem_wq, sem_ax, sem_out):
    cp = pltpu.make_async_copy

    c_w1 = cp(w1_hbm, w1, sem_w.at[0])
    c_gw = cp(gw_hbm, gw, sem_w.at[1])
    late = (
        cp(wqkv_hbm.at[:, pl.ds(2 * D, D)], wv, sem_w.at[2]),
        cp(wo_hbm, wo, sem_w.at[3]),
        cp(w2_hbm, w2, sem_w.at[4]),
        cp(w3t_hbm, w3t, sem_w.at[5]),
        cp(w4_hbm, w4, sem_w.at[6]),
    )

    def c_wk(j):
        lo, hi = WK_PIECES[j]
        return cp(wqkv_hbm.at[:, pl.ds(D + lo, hi - lo)], wk.at[:, pl.ds(lo, hi - lo)], sem_wk.at[j])

    def c_wq(j):
        src = min(j, NT - 1) if isinstance(j, int) else jnp.minimum(j, NT - 1)
        return cp(wqkv_hbm.at[:, pl.ds(_al(128 * src, 128), 128)], wq.at[j], sem_wq.at[j])

    def c_ax(i):
        return cp(ax_hbm.at[0, pl.ds(i * XC, XC), :], ax.at[pl.ds(i * XC, XC), :], sem_ax.at[i])

    def c_out(i):
        return cp(obuf.at[pl.ds(i * T2, T2), :], out_hbm.at[0, pl.ds(i * T2, T2), :], sem_out.at[i])

    def start_trip(t):
        for c in range(CPT):
            c_ax(2 + t * CPT + c).start()
        for c in range(WPT):
            c_wq(t * WPT + c).start()

    c_ax(0).start()
    for j in range(len(WK_PIECES)):
        c_wk(j).start()
    c_ax(1).start()

    zeros8 = jnp.zeros((HALO, 128), F32)
    for j in range(NT):
        h_scr[j, 0:HALO, :] = zeros8
        h_scr[j, HALO + S:HALO + S + HALO, :] = zeros8
    z_scr[...] = jnp.zeros((PADROWS, 128), F32)

    def k_post(k, c0):
        rows = k.shape[0]
        pkT = _phi(k).T
        acc = pkT[:, 0:128]
        for t in range(1, rows // 128):
            acc = acc + pkT[:, 128 * t:128 * (t + 1)]
        z_scr[0:D, :] += acc
        pkt[:, c0:c0 + rows] = pkT.astype(BF16)

    def mix_pre(r0):
        xf = ax[pl.ds(r0, T1), :].astype(F32)
        return _dot(_ln(xf).astype(BF16), w1[...])

    def mix_post(hpre, r0):
        h = _gelu(hpre)
        for j in range(NT):
            h_scr[j, pl.ds(r0 + HALO, T1), :] = h[:, 128 * j:128 * (j + 1)]

    def wq_t_chunk(j):
        wqT = wq[j].astype(F32).T
        for n in range(NT):
            t_scr[n, pl.ds(_al(128 * j, 128), 128), :] = wqT[:, 128 * n:128 * (n + 1)]

    c_ax(0).wait()
    c_wk(0).wait()
    c_w1.start()
    c_gw.start()
    xa0 = ax[0:XC, :]
    parts = []
    for j, (lo, hi) in enumerate(WK_PIECES):
        if j > 0:
            c_wk(j).wait()
        if j == len(WK_PIECES) - 1:
            start_trip(0)
        tiles = NT * (hi - lo) // 128
        parts.append(_dot_rows(xa0, wk[:, lo:hi], 2 if tiles % 2 == 0 else 4))
    k0 = jnp.concatenate(parts, axis=1)
    c_ax(1).wait()
    for t in range(1, NL):
        start_trip(t)
    for c in late:
        c.start(priority=1)
    k1a = _dot(ax[XC:XC + 128, :], wk[...])
    k_post(k0, 0)
    k1b = _dot(ax[XC + 128:R0, :], wk[...])
    k_post(k1a, XC)
    k_post(k1b, XC + 128)
    g_scr[...] = _dot(pkt[:, 0:R0], ax[0:R0, :])
    c_w1.wait()
    c_gw.wait()
    gwf[...] = gw[...].astype(F32).reshape(1, D)

    def phase1(t, carry):
        ra = _al(R0 + t * RL, XC)
        rb = _al(t * RL, XC)
        for c in range(CPT):
            c_ax(2 + t * CPT + c).wait()
        for c in range(WPT):
            c_wq(t * WPT + c).wait()
        for s in range(NS1):
            k = _dot(ax[pl.ds(ra + s * T1, T1), :], wk[...])
            hpre = mix_pre(rb + s * T1)
            k_post(k, s * T1)
            mix_post(hpre, rb + s * T1)
            if s < WPT:
                wq_t_chunk(t * WPT + s)
        g_scr[...] += _dot(pkt[...], ax[pl.ds(ra, RL), :])
        return carry

    lax.fori_loop(0, NL, phase1, 0)

    for c in late:
        c.wait()

    def m_build(kvs):
        prev = None
        for j, (lo, hi) in enumerate(KV_ROWS):
            rh = (lax.broadcasted_iota(jnp.int32, (hi - lo, 128), 0) + lo) // DH
            ch = (lax.broadcasted_iota(jnp.int32, (hi - lo, 128), 1) + 128 * j) // DH
            kv = jnp.where(rh == ch, kvs[j], 0.0).astype(BF16)
            mj = _dot(kv, wo[128 * j:128 * (j + 1), :])
            ov = 0 if prev is None else prev.shape[0]
            nxt = KV_ROWS[j + 1][0] if j + 1 < NT else hi
            for n in range(NT):
                col = mj[:, 128 * n:128 * (n + 1)]
                if ov:
                    m_scr[n, lo:lo + ov, :] = col[0:ov] + prev[:, 128 * n:128 * (n + 1)]
                m_scr[n, lo + ov:nxt, :] = col[ov:nxt - lo]
            prev = mj[nxt - lo:, :] if j + 1 < NT else None

    def gather(dst, src):
        for d in range(DH):
            for n in range(NT):
                dst[H * d:H * (d + 1), 128 * n:128 * (n + 1)] = (
                    src[n, pl.ds(d, H, stride=DH), :].astype(BF16))

    def gather_z():
        zp = jnp.concatenate([z_scr[pl.ds(d, H, stride=DH), :] for d in range(DH)], axis=0)
        zrow[...] = jnp.sum(zp.T, axis=0, keepdims=True)

    rb = S - R0
    kvs = [_dot(g_scr[lo:hi, :].astype(BF16), wv[:, 128 * j:128 * (j + 1)])
           for j, (lo, hi) in enumerate(KV_ROWS)]
    hpre = mix_pre(rb)
    m_build(kvs)
    extra = [lambda: gather(wqp, t_scr), lambda: gather(mp, m_scr), gather_z]
    for s in range(R0 // T1):
        nxt_pre = mix_pre(rb + (s + 1) * T1) if s + 1 < R0 // T1 else None
        mix_post(hpre, rb + s * T1)
        if s < len(extra):
            extra[s]()
        hpre = nxt_pre

    lane = lax.broadcasted_iota(jnp.int32, (T2, 128), 1)

    def st_q(i):
        return _dot_nt(ax[pl.ds(_al(i * T2, T2), T2), :], wqp[...])

    def st_w2(i):
        r0 = _al(i * T2, T2)

        def hrow(j, off):
            return h_scr[j, pl.ds(r0 + HALO + off, T2), :]

        hs = jnp.concatenate([
            hrow(0, -1),
            jnp.where(lane < 32, hrow(1, -1), hrow(1, 1)),
            jnp.where(lane < 64, hrow(2, 1), hrow(2, -2)),
            jnp.where(lane < 96, hrow(3, -2), hrow(3, 2)),
            hrow(4, 2),
        ], axis=1).astype(BF16)
        return _dot(hs, w2[...])

    def st_phi(i, q):
        pq = _phi(q)
        pz = pq * zrow[...]
        den = pz[:, 0:128]
        for t in range(1, NT):
            den = den + pz[:, 128 * t:128 * (t + 1)]
        den = den + pltpu.roll(den, 64, 1)
        den = den + pltpu.roll(den, 32, 1)
        xf = ax[pl.ds(_al(i * T2, T2), T2), :].astype(F32)
        g = jax.nn.sigmoid(jnp.sum(xf * gwf[...], axis=-1, keepdims=True))
        r = g / (den + 1e-6)
        pqn = jnp.concatenate([pq[:, 128 * t:128 * (t + 1)] * r for t in range(NT)], axis=1)
        return pqn.astype(BF16), 1.0 - g

    def st_ln2(i, y):
        x1 = ax[pl.ds(_al(i * T2, T2), T2), :].astype(F32) + y
        return x1, _ln(x1).astype(BF16)

    def st_w3(ln2):
        u_main = _gelu(_dot_nt(ln2, w3t[0:FM, :])).astype(BF16)
        u_last = _gelu(_dot_nt(w3t[FM:FF, :], ln2)).T.astype(BF16)
        return jnp.concatenate([u_main, u_last], axis=1)

    def phase2(trip, carry):
        i0 = trip * U2
        q = st_q(i0)
        y = st_w2(i0)
        pqn, omg = st_phi(i0, q)
        a = _dot(pqn, mp[...])
        x1, ln2 = st_ln2(i0, y)
        for u in range(U2):
            i = i0 + u
            more = u + 1 < U2
            if more:
                q = st_q(i + 1)
            base = a + omg * x1
            omg_i = omg
            uu = st_w3(ln2)
            if more:
                y = st_w2(i + 1)
                pqn, omg = st_phi(i + 1, q)
            h2 = _dot(uu, w4[...])
            if more:
                x1, ln2 = st_ln2(i + 1, y)
                a = _dot(pqn, mp[...])
            obuf[pl.ds(_al(i * T2, T2), T2), :] = (base + omg_i * h2).astype(BF16)
            c_out(i).start()
        return carry

    lax.fori_loop(0, N2 // U2, phase2, 0)
    for i in range(N2):
        c_out(i).wait()


_SCRATCH = [
    pltpu.VMEM((S, D), BF16),
    pltpu.VMEM((NT + 1, D, 128), BF16),
    pltpu.VMEM((D, D), BF16),
    pltpu.VMEM((D, D), BF16),
    pltpu.VMEM((D, D), BF16),
    pltpu.VMEM((D, D), BF16),
    pltpu.VMEM((D, D), BF16),
    pltpu.VMEM((FF, D), BF16),
    pltpu.VMEM((FF, D), BF16),
    pltpu.VMEM((D,), BF16),
    pltpu.VMEM((1, D), F32),
    pltpu.VMEM((NT, S + 2 * HALO, 128), F32),
    pltpu.VMEM((D, D), F32),
    pltpu.VMEM((PADROWS, 128), F32),
    pltpu.VMEM((NT, PADROWS, 128), F32),
    pltpu.VMEM((NT, 128 * (NT + 1), 128), F32),
    pltpu.VMEM((D, D), BF16),
    pltpu.VMEM((D, D), BF16),
    pltpu.VMEM((1, D), F32),
    pltpu.VMEM((D, RL), BF16),
    pltpu.VMEM((S, D), BF16),
    pltpu.SemaphoreType.DMA((7,)),
    pltpu.SemaphoreType.DMA((len(WK_PIECES),)),
    pltpu.SemaphoreType.DMA((NT + 1,)),
    pltpu.SemaphoreType.DMA((NXC,)),
    pltpu.SemaphoreType.DMA((N2,)),
]


@jax.jit
def pallas_gated_mix__linear_attn_block__mixer_s_mlp__prompt_kernel(
    A_x: jax.Array,
    A_wqkv: jax.Array,
    A_wo: jax.Array,
    B_x: jax.Array,
    B_w1: jax.Array,
    B_w2: jax.Array,
    B_w3: jax.Array,
    B_w4: jax.Array,
    gate_w: jax.Array,
):
    del B_x
    return pl.pallas_call(
        _kernel,
        out_shape=jax.ShapeDtypeStruct((1, S, D), BF16),
        in_specs=[pl.BlockSpec(memory_space=pl.ANY)] * 8,
        out_specs=pl.BlockSpec(memory_space=pl.ANY),
        scratch_shapes=_SCRATCH,
        compiler_params=pltpu.CompilerParams(vmem_limit_bytes=100 * 2**20),
    )(A_x, A_wqkv, A_wo, B_w1, B_w2, B_w3.T, B_w4, gate_w)
```

```python
import jax
import jax.numpy as jnp
from jax import lax
from jax.experimental import pallas as pl
from jax.experimental.pallas import tpu as pltpu

F32 = jnp.float32
BF16 = jnp.bfloat16

S, D, FF = 2048, 640, 1728
H, DH = 32, 20
NT = D // 128
HALO = 8
KV_ROWS = ((0, 144), (120, 264), (240, 400), (376, 520), (496, 640))
PADROWS = 672
XC = 256
NXC = S // XC
R0 = 2 * XC
RL = 512
NL = (S - R0) // RL
CPT = RL // XC
WPT = (NT + 1) // NL
T1 = 128
NS1 = RL // T1
T2 = 128
U2 = 4
N2 = S // T2
FM = 1664
FH = 896
WK_PIECES = ((0, 128), (128, 384), (384, D))


def _gelu(x):
    c0 = 0.7978845608028654
    c1 = 0.7978845608028654 * 0.044715
    u = x * (c0 + c1 * (x * x))
    hx = 0.5 * x
    return hx + hx * jnp.tanh(u)


def _phi(t):
    return jnp.where(t > 0, t + 1.0, jnp.exp(t)) + 1e-6


def _ln(x):
    m = jnp.mean(x, axis=-1, keepdims=True)
    xc = x - m
    v = jnp.mean(xc * xc, axis=-1, keepdims=True)
    return xc * lax.rsqrt(v + 1e-5)


def _dot(a, b):
    return jnp.dot(a, b, preferred_element_type=F32)


def _dot_nt(a, b):
    return lax.dot_general(a, b, (((1,), (1,)), ((), ())), preferred_element_type=F32)


def _dot_rows(a, b, parts):
    n = a.shape[0] // parts
    return jnp.concatenate([_dot(a[p * n:(p + 1) * n, :], b) for p in range(parts)], axis=0)


def _al(x, m):
    return x if isinstance(x, int) else pl.multiple_of(x, m)


def _kernel(ax_hbm, wqkv_hbm, wo_hbm, w1_hbm, w2_hbm, w3t_hbm, w4_hbm, gw_hbm,
            out_hbm,
            ax, wq, wk, wv, wo, w1, w2, w3t, w4, gw, gwf,
            h_scr, g_scr, z_scr, m_scr, t_scr, mp, wqp, zrow, pkt, obuf,
            sem_w, sem_wk, sem_wq, sem_ax, sem_out):
    cp = pltpu.make_async_copy

    c_w1 = cp(w1_hbm, w1, sem_w.at[0])
    c_gw = cp(gw_hbm, gw, sem_w.at[1])
    late = (
        cp(wqkv_hbm.at[:, pl.ds(2 * D, D)], wv, sem_w.at[2]),
        cp(wo_hbm, wo, sem_w.at[3]),
        cp(w2_hbm, w2, sem_w.at[4]),
        cp(w3t_hbm, w3t, sem_w.at[5]),
        cp(w4_hbm, w4, sem_w.at[6]),
    )

    def c_wk(j):
        lo, hi = WK_PIECES[j]
        return cp(wqkv_hbm.at[:, pl.ds(D + lo, hi - lo)], wk.at[:, pl.ds(lo, hi - lo)], sem_wk.at[j])

    def c_wq(j):
        src = min(j, NT - 1) if isinstance(j, int) else jnp.minimum(j, NT - 1)
        return cp(wqkv_hbm.at[:, pl.ds(_al(128 * src, 128), 128)], wq.at[j], sem_wq.at[j])

    def c_ax(i):
        return cp(ax_hbm.at[0, pl.ds(i * XC, XC), :], ax.at[pl.ds(i * XC, XC), :], sem_ax.at[i])

    def c_out(i):
        return cp(obuf.at[pl.ds(i * T2, T2), :], out_hbm.at[0, pl.ds(i * T2, T2), :], sem_out.at[i])

    def start_trip(t):
        for c in range(CPT):
            c_ax(2 + t * CPT + c).start()
        for c in range(WPT):
            c_wq(t * WPT + c).start()

    c_ax(0).start()
    for j in range(len(WK_PIECES)):
        c_wk(j).start()
    c_ax(1).start()

    zeros8 = jnp.zeros((HALO, 128), F32)
    for j in range(NT):
        h_scr[j, 0:HALO, :] = zeros8
        h_scr[j, HALO + S:HALO + S + HALO, :] = zeros8
    z_scr[...] = jnp.zeros((PADROWS, 128), F32)

    def k_post(k, c0):
        rows = k.shape[0]
        pkT = _phi(k).T
        acc = pkT[:, 0:128]
        for t in range(1, rows // 128):
            acc = acc + pkT[:, 128 * t:128 * (t + 1)]
        z_scr[0:D, :] += acc
        pkt[:, c0:c0 + rows] = pkT.astype(BF16)

    def mix_pre(r0):
        xf = ax[pl.ds(r0, T1), :].astype(F32)
        return _dot(_ln(xf).astype(BF16), w1[...])

    def mix_post(hpre, r0):
        h = _gelu(hpre)
        for j in range(NT):
            h_scr[j, pl.ds(r0 + HALO, T1), :] = h[:, 128 * j:128 * (j + 1)]

    def wq_t_chunk(j):
        wqT = wq[j].astype(F32).T
        for n in range(NT):
            t_scr[n, pl.ds(_al(128 * j, 128), 128), :] = wqT[:, 128 * n:128 * (n + 1)]

    c_ax(0).wait()
    c_wk(0).wait()
    c_w1.start()
    c_gw.start()
    xa0 = ax[0:XC, :]
    parts = []
    for j, (lo, hi) in enumerate(WK_PIECES):
        if j > 0:
            c_wk(j).wait()
        if j == len(WK_PIECES) - 1:
            start_trip(0)
        tiles = NT * (hi - lo) // 128
        parts.append(_dot_rows(xa0, wk[:, lo:hi], 2 if tiles % 2 == 0 else 4))
    k0 = jnp.concatenate(parts, axis=1)
    c_ax(1).wait()
    for t in range(1, NL):
        start_trip(t)
    for c in late:
        c.start(priority=1)
    k1a = _dot(ax[XC:XC + 128, :], wk[...])
    k_post(k0, 0)
    k1b = _dot(ax[XC + 128:R0, :], wk[...])
    k_post(k1a, XC)
    k_post(k1b, XC + 128)
    g_scr[...] = _dot(pkt[:, 0:R0], ax[0:R0, :])
    c_w1.wait()
    c_gw.wait()
    gwf[...] = gw[...].astype(F32).reshape(1, D)

    def phase1(t, carry):
        ra = _al(R0 + t * RL, XC)
        rb = _al(t * RL, XC)
        for c in range(CPT):
            c_ax(2 + t * CPT + c).wait()
        for c in range(WPT):
            c_wq(t * WPT + c).wait()
        for s in range(NS1):
            k = _dot(ax[pl.ds(ra + s * T1, T1), :], wk[...])
            hpre = mix_pre(rb + s * T1)
            k_post(k, s * T1)
            mix_post(hpre, rb + s * T1)
            if s < WPT:
                wq_t_chunk(t * WPT + s)
        g_scr[...] += _dot(pkt[...], ax[pl.ds(ra, RL), :])
        return carry

    lax.fori_loop(0, NL, phase1, 0)

    for c in late:
        c.wait()

    def m_build(kvs):
        prev = None
        for j, (lo, hi) in enumerate(KV_ROWS):
            rh = (lax.broadcasted_iota(jnp.int32, (hi - lo, 128), 0) + lo) // DH
            ch = (lax.broadcasted_iota(jnp.int32, (hi - lo, 128), 1) + 128 * j) // DH
            kv = jnp.where(rh == ch, kvs[j], 0.0).astype(BF16)
            mj = _dot(kv, wo[128 * j:128 * (j + 1), :])
            ov = 0 if prev is None else prev.shape[0]
            nxt = KV_ROWS[j + 1][0] if j + 1 < NT else hi
            for n in range(NT):
                col = mj[:, 128 * n:128 * (n + 1)]
                if ov:
                    m_scr[n, lo:lo + ov, :] = col[0:ov] + prev[:, 128 * n:128 * (n + 1)]
                m_scr[n, lo + ov:nxt, :] = col[ov:nxt - lo]
            prev = mj[nxt - lo:, :] if j + 1 < NT else None

    def gather(dst, src):
        for d in range(DH):
            for n in range(NT):
                dst[H * d:H * (d + 1), 128 * n:128 * (n + 1)] = (
                    src[n, pl.ds(d, H, stride=DH), :].astype(BF16))

    def gather_z():
        zp = jnp.concatenate([z_scr[pl.ds(d, H, stride=DH), :] for d in range(DH)], axis=0)
        zrow[...] = jnp.sum(zp.T, axis=0, keepdims=True)

    rb = S - R0
    kvs = [_dot(g_scr[lo:hi, :].astype(BF16), wv[:, 128 * j:128 * (j + 1)])
           for j, (lo, hi) in enumerate(KV_ROWS)]
    hpre = mix_pre(rb)
    m_build(kvs)
    extra = [lambda: gather(wqp, t_scr), lambda: gather(mp, m_scr), gather_z]
    for s in range(R0 // T1):
        nxt_pre = mix_pre(rb + (s + 1) * T1) if s + 1 < R0 // T1 else None
        mix_post(hpre, rb + s * T1)
        if s < len(extra):
            extra[s]()
        hpre = nxt_pre

    lane = lax.broadcasted_iota(jnp.int32, (T2, 128), 1)

    def st_q(i):
        return _dot_nt(ax[pl.ds(_al(i * T2, T2), T2), :], wqp[...])

    def st_w2(i):
        r0 = _al(i * T2, T2)

        def hrow(j, off):
            return h_scr[j, pl.ds(r0 + HALO + off, T2), :]

        hs = jnp.concatenate([
            hrow(0, -1),
            jnp.where(lane < 32, hrow(1, -1), hrow(1, 1)),
            jnp.where(lane < 64, hrow(2, 1), hrow(2, -2)),
            jnp.where(lane < 96, hrow(3, -2), hrow(3, 2)),
            hrow(4, 2),
        ], axis=1).astype(BF16)
        return _dot(hs, w2[...])

    def st_phi(i, q):
        pq = _phi(q)
        pz = pq * zrow[...]
        den = pz[:, 0:128]
        for t in range(1, NT):
            den = den + pz[:, 128 * t:128 * (t + 1)]
        den = den + pltpu.roll(den, 64, 1)
        den = den + pltpu.roll(den, 32, 1)
        xf = ax[pl.ds(_al(i * T2, T2), T2), :].astype(F32)
        g = jax.nn.sigmoid(jnp.sum(xf * gwf[...], axis=-1, keepdims=True))
        r = g / (den + 1e-6)
        pqn = jnp.concatenate([pq[:, 128 * t:128 * (t + 1)] * r for t in range(NT)], axis=1)
        return pqn.astype(BF16), 1.0 - g

    def st_ln2(i, y):
        x1 = ax[pl.ds(_al(i * T2, T2), T2), :].astype(F32) + y
        return x1, _ln(x1).astype(BF16)

    def st_w3(ln2):
        u_a = _gelu(_dot_nt(ln2, w3t[0:FH, :])).astype(BF16)
        u_last = _gelu(_dot_nt(w3t[FM:FF, :], ln2)).T.astype(BF16)
        u_b = _gelu(_dot_nt(ln2, w3t[FH:FM, :])).astype(BF16)
        return jnp.concatenate([u_a, u_b, u_last], axis=1)

    def phase2(trip, carry):
        i0 = trip * U2
        q = st_q(i0)
        y = st_w2(i0)
        pqn, omg = st_phi(i0, q)
        a = _dot(pqn, mp[...])
        x1, ln2 = st_ln2(i0, y)
        for u in range(U2):
            i = i0 + u
            more = u + 1 < U2
            if more:
                q = st_q(i + 1)
            base = a + omg * x1
            omg_i = omg
            uu = st_w3(ln2)
            if more:
                y = st_w2(i + 1)
                pqn, omg = st_phi(i + 1, q)
            h2 = _dot(uu, w4[...])
            if more:
                x1, ln2 = st_ln2(i + 1, y)
                a = _dot(pqn, mp[...])
            obuf[pl.ds(_al(i * T2, T2), T2), :] = (base + omg_i * h2).astype(BF16)
            c_out(i).start()
        return carry

    lax.fori_loop(0, N2 // U2, phase2, 0)
    for i in range(N2):
        c_out(i).wait()


_SCRATCH = [
    pltpu.VMEM((S, D), BF16),
    pltpu.VMEM((NT + 1, D, 128), BF16),
    pltpu.VMEM((D, D), BF16),
    pltpu.VMEM((D, D), BF16),
    pltpu.VMEM((D, D), BF16),
    pltpu.VMEM((D, D), BF16),
    pltpu.VMEM((D, D), BF16),
    pltpu.VMEM((FF, D), BF16),
    pltpu.VMEM((FF, D), BF16),
    pltpu.VMEM((D,), BF16),
    pltpu.VMEM((1, D), F32),
    pltpu.VMEM((NT, S + 2 * HALO, 128), F32),
    pltpu.VMEM((D, D), F32),
    pltpu.VMEM((PADROWS, 128), F32),
    pltpu.VMEM((NT, PADROWS, 128), F32),
    pltpu.VMEM((NT, 128 * (NT + 1), 128), F32),
    pltpu.VMEM((D, D), BF16),
    pltpu.VMEM((D, D), BF16),
    pltpu.VMEM((1, D), F32),
    pltpu.VMEM((D, RL), BF16),
    pltpu.VMEM((S, D), BF16),
    pltpu.SemaphoreType.DMA((7,)),
    pltpu.SemaphoreType.DMA((len(WK_PIECES),)),
    pltpu.SemaphoreType.DMA((NT + 1,)),
    pltpu.SemaphoreType.DMA((NXC,)),
    pltpu.SemaphoreType.DMA((N2,)),
]


@jax.jit
def pallas_gated_mix__linear_attn_block__mixer_s_mlp__prompt_kernel(
    A_x: jax.Array,
    A_wqkv: jax.Array,
    A_wo: jax.Array,
    B_x: jax.Array,
    B_w1: jax.Array,
    B_w2: jax.Array,
    B_w3: jax.Array,
    B_w4: jax.Array,
    gate_w: jax.Array,
):
    del B_x
    return pl.pallas_call(
        _kernel,
        out_shape=jax.ShapeDtypeStruct((1, S, D), BF16),
        in_specs=[pl.BlockSpec(memory_space=pl.ANY)] * 8,
        out_specs=pl.BlockSpec(memory_space=pl.ANY),
        scratch_shapes=_SCRATCH,
        compiler_params=pltpu.CompilerParams(vmem_limit_bytes=100 * 2**20),
    )(A_x, A_wqkv, A_wo, B_w1, B_w2, B_w3.T, B_w4, gate_w)
```

```python
import jax
import jax.numpy as jnp
from jax import lax
from jax.experimental import pallas as pl
from jax.experimental.pallas import tpu as pltpu

F32 = jnp.float32
BF16 = jnp.bfloat16

S, D, FF = 2048, 640, 1728
H, DH = 32, 20
NT = D // 128
HALO = 8
KV_ROWS = ((0, 144), (120, 264), (240, 400), (376, 520), (496, 640))
PADROWS = 672
XC = 256
NXC = S // XC
R0 = 2 * XC
RL = 512
NL = (S - R0) // RL
CPT = RL // XC
WPT = (NT + 1) // NL
T1 = 128
NS1 = RL // T1
T2 = 128
U2 = 4
N2 = S // T2
FM = 1664
FH = 896
WK_PIECES = ((0, 128), (128, 384), (384, D))


def _gelu(x):
    c0 = 0.7978845608028654
    c1 = 0.7978845608028654 * 0.044715
    u = x * (c0 + c1 * (x * x))
    hx = 0.5 * x
    return hx + hx * jnp.tanh(u)


def _phi(t):
    return jnp.where(t > 0, t + 1.0, jnp.exp(t)) + 1e-6


def _ln(x):
    m = jnp.mean(x, axis=-1, keepdims=True)
    xc = x - m
    v = jnp.mean(xc * xc, axis=-1, keepdims=True)
    return xc * lax.rsqrt(v + 1e-5)


def _dot(a, b):
    return jnp.dot(a, b, preferred_element_type=F32)


def _dot_nt(a, b):
    return lax.dot_general(a, b, (((1,), (1,)), ((), ())), preferred_element_type=F32)


def _dot_rows(a, b, parts):
    n = a.shape[0] // parts
    return jnp.concatenate([_dot(a[p * n:(p + 1) * n, :], b) for p in range(parts)], axis=0)


def _al(x, m):
    return x if isinstance(x, int) else pl.multiple_of(x, m)


def _kernel(ax_hbm, wqkv_hbm, wo_hbm, w1_hbm, w2_hbm, w3t_hbm, w4_hbm, gw_hbm,
            out_hbm,
            ax, wq, wk, wv, wo, w1, w2, w3t, w4, gw, gwf,
            h_scr, g_scr, z_scr, m_scr, t_scr, mp, wqp, zrow, pkt, obuf,
            sem_w, sem_wk, sem_wq, sem_ax, sem_out):
    cp = pltpu.make_async_copy

    c_w1 = cp(w1_hbm, w1, sem_w.at[0])
    c_gw = cp(gw_hbm, gw, sem_w.at[1])
    late = (
        cp(wqkv_hbm.at[:, pl.ds(2 * D, D)], wv, sem_w.at[2]),
        cp(wo_hbm, wo, sem_w.at[3]),
        cp(w2_hbm, w2, sem_w.at[4]),
        cp(w3t_hbm, w3t, sem_w.at[5]),
        cp(w4_hbm, w4, sem_w.at[6]),
    )

    def c_wk(j):
        lo, hi = WK_PIECES[j]
        return cp(wqkv_hbm.at[:, pl.ds(D + lo, hi - lo)], wk.at[:, pl.ds(lo, hi - lo)], sem_wk.at[j])

    def c_wq(j):
        src = min(j, NT - 1) if isinstance(j, int) else jnp.minimum(j, NT - 1)
        return cp(wqkv_hbm.at[:, pl.ds(_al(128 * src, 128), 128)], wq.at[j], sem_wq.at[j])

    def c_ax(i):
        return cp(ax_hbm.at[0, pl.ds(i * XC, XC), :], ax.at[pl.ds(i * XC, XC), :], sem_ax.at[i])

    def c_out(i):
        return cp(obuf.at[pl.ds(i * T2, T2), :], out_hbm.at[0, pl.ds(i * T2, T2), :], sem_out.at[i])

    def start_trip(t):
        for c in range(CPT):
            c_ax(2 + t * CPT + c).start()
        for c in range(WPT):
            c_wq(t * WPT + c).start()

    c_ax(0).start()
    for j in range(len(WK_PIECES)):
        c_wk(j).start()
    c_ax(1).start()

    zeros8 = jnp.zeros((HALO, 128), F32)
    for j in range(NT):
        h_scr[j, 0:HALO, :] = zeros8
        h_scr[j, HALO + S:HALO + S + HALO, :] = zeros8
    z_scr[...] = jnp.zeros((PADROWS, 128), F32)

    def k_post(k, c0):
        rows = k.shape[0]
        pkT = _phi(k).T
        acc = pkT[:, 0:128]
        for t in range(1, rows // 128):
            acc = acc + pkT[:, 128 * t:128 * (t + 1)]
        z_scr[0:D, :] += acc
        pkt[:, c0:c0 + rows] = pkT.astype(BF16)

    def mix_pre(r0):
        xf = ax[pl.ds(r0, T1), :].astype(F32)
        return _dot(_ln(xf).astype(BF16), w1[...])

    def mix_post(hpre, r0):
        h = _gelu(hpre)
        for j in range(NT):
            h_scr[j, pl.ds(r0 + HALO, T1), :] = h[:, 128 * j:128 * (j + 1)]

    def wq_t_chunk(j):
        wqT = wq[j].astype(F32).T
        for n in range(NT):
            t_scr[n, pl.ds(_al(128 * j, 128), 128), :] = wqT[:, 128 * n:128 * (n + 1)]

    c_ax(0).wait()
    c_wk(0).wait()
    c_w1.start()
    c_gw.start()
    xa0 = ax[0:XC, :]
    parts = []
    for j, (lo, hi) in enumerate(WK_PIECES):
        if j > 0:
            c_wk(j).wait()
        if j == len(WK_PIECES) - 1:
            start_trip(0)
        tiles = NT * (hi - lo) // 128
        parts.append(_dot_rows(xa0, wk[:, lo:hi], 2 if tiles % 2 == 0 else 4))
    k0 = jnp.concatenate(parts, axis=1)
    c_ax(1).wait()
    for t in range(1, NL):
        start_trip(t)
    for c in late:
        c.start(priority=1)
    k1a = _dot(ax[XC:XC + 128, :], wk[...])
    k_post(k0, 0)
    k1b = _dot(ax[XC + 128:R0, :], wk[...])
    k_post(k1a, XC)
    k_post(k1b, XC + 128)
    g_scr[...] = _dot(pkt[:, 0:R0], ax[0:R0, :])
    c_w1.wait()
    c_gw.wait()
    gwf[...] = gw[...].astype(F32).reshape(1, D)

    def phase1(t, carry):
        ra = _al(R0 + t * RL, XC)
        rb = _al(t * RL, XC)
        for c in range(CPT):
            c_ax(2 + t * CPT + c).wait()
        for c in range(WPT):
            c_wq(t * WPT + c).wait()
        for s in range(NS1):
            k = _dot(ax[pl.ds(ra + s * T1, T1), :], wk[...])
            hpre = mix_pre(rb + s * T1)
            k_post(k, s * T1)
            mix_post(hpre, rb + s * T1)
            if s < WPT:
                wq_t_chunk(t * WPT + s)
        g_scr[...] += _dot(pkt[...], ax[pl.ds(ra, RL), :])
        return carry

    lax.fori_loop(0, NL, phase1, 0)

    for c in late:
        c.wait()

    def m_build(kvs):
        prev = None
        for j, (lo, hi) in enumerate(KV_ROWS):
            col = lax.broadcasted_iota(jnp.int32, (8, 128), 1) + 128 * j
            first = ((col * 3277) >> 16) * DH - lo
            first = jnp.concatenate([first] * ((hi - lo) // 8), axis=0)
            off = lax.broadcasted_iota(jnp.int32, (hi - lo, 128), 0) - first
            kv = jnp.where((off >= 0) & (off < DH), kvs[j], 0.0).astype(BF16)
            mj = _dot(kv, wo[128 * j:128 * (j + 1), :])
            ov = 0 if prev is None else prev.shape[0]
            nxt = KV_ROWS[j + 1][0] if j + 1 < NT else hi
            for n in range(NT):
                blk = mj[:, 128 * n:128 * (n + 1)]
                if ov:
                    m_scr[n, lo:lo + ov, :] = blk[0:ov] + prev[:, 128 * n:128 * (n + 1)]
                m_scr[n, lo + ov:nxt, :] = blk[ov:nxt - lo]
            prev = mj[nxt - lo:, :] if j + 1 < NT else None

    def gather(dst, src):
        for d in range(DH):
            for n in range(NT):
                dst[H * d:H * (d + 1), 128 * n:128 * (n + 1)] = (
                    src[n, pl.ds(d, H, stride=DH), :].astype(BF16))

    def gather_z():
        zp = jnp.concatenate([z_scr[pl.ds(d, H, stride=DH), :] for d in range(DH)], axis=0)
        zrow[...] = jnp.sum(zp.T, axis=0, keepdims=True)

    rb = S - R0
    kvs = [_dot(g_scr[lo:hi, :].astype(BF16), wv[:, 128 * j:128 * (j + 1)])
           for j, (lo, hi) in enumerate(KV_ROWS)]
    hpre = mix_pre(rb)
    m_build(kvs)
    extra = [lambda: gather(wqp, t_scr), lambda: gather(mp, m_scr), gather_z]
    for s in range(R0 // T1):
        nxt_pre = mix_pre(rb + (s + 1) * T1) if s + 1 < R0 // T1 else None
        mix_post(hpre, rb + s * T1)
        if s < len(extra):
            extra[s]()
        hpre = nxt_pre

    lane = lax.broadcasted_iota(jnp.int32, (T2, 128), 1)

    def st_q(i):
        return _dot_nt(ax[pl.ds(_al(i * T2, T2), T2), :], wqp[...])

    def st_w2(i):
        r0 = _al(i * T2, T2)

        def hrow(j, off):
            return h_scr[j, pl.ds(r0 + HALO + off, T2), :]

        hs = jnp.concatenate([
            hrow(0, -1),
            jnp.where(lane < 32, hrow(1, -1), hrow(1, 1)),
            jnp.where(lane < 64, hrow(2, 1), hrow(2, -2)),
            jnp.where(lane < 96, hrow(3, -2), hrow(3, 2)),
            hrow(4, 2),
        ], axis=1).astype(BF16)
        return _dot(hs, w2[...])

    def st_phi(i, q):
        pq = _phi(q)
        pz = pq * zrow[...]
        den = pz[:, 0:128]
        for t in range(1, NT):
            den = den + pz[:, 128 * t:128 * (t + 1)]
        den = den + pltpu.roll(den, 64, 1)
        den = den + pltpu.roll(den, 32, 1)
        xf = ax[pl.ds(_al(i * T2, T2), T2), :].astype(F32)
        g = jax.nn.sigmoid(jnp.sum(xf * gwf[...], axis=-1, keepdims=True))
        r = g / (den + 1e-6)
        pqn = jnp.concatenate([pq[:, 128 * t:128 * (t + 1)] * r for t in range(NT)], axis=1)
        return pqn.astype(BF16), 1.0 - g

    def st_ln2(i, y):
        x1 = ax[pl.ds(_al(i * T2, T2), T2), :].astype(F32) + y
        return x1, _ln(x1).astype(BF16)

    def st_w3(ln2):
        u_a = _gelu(_dot_nt(ln2, w3t[0:FH, :])).astype(BF16)
        u_last = _gelu(_dot_nt(w3t[FM:FF, :], ln2)).T.astype(BF16)
        u_b = _gelu(_dot_nt(ln2, w3t[FH:FM, :])).astype(BF16)
        return jnp.concatenate([u_a, u_b, u_last], axis=1)

    def phase2(trip, carry):
        i0 = trip * U2
        q = st_q(i0)
        y = st_w2(i0)
        pqn, omg = st_phi(i0, q)
        a = _dot(pqn, mp[...])
        x1, ln2 = st_ln2(i0, y)
        for u in range(U2):
            i = i0 + u
            more = u + 1 < U2
            if more:
                q = st_q(i + 1)
            base = a + omg * x1
            omg_i = omg
            uu = st_w3(ln2)
            if more:
                y = st_w2(i + 1)
                pqn, omg = st_phi(i + 1, q)
            h2 = _dot(uu, w4[...])
            if more:
                x1, ln2 = st_ln2(i + 1, y)
                a = _dot(pqn, mp[...])
            obuf[pl.ds(_al(i * T2, T2), T2), :] = (base + omg_i * h2).astype(BF16)
            c_out(i).start()
        return carry

    lax.fori_loop(0, N2 // U2, phase2, 0)
    for i in range(N2):
        c_out(i).wait()


_SCRATCH = [
    pltpu.VMEM((S, D), BF16),
    pltpu.VMEM((NT + 1, D, 128), BF16),
    pltpu.VMEM((D, D), BF16),
    pltpu.VMEM((D, D), BF16),
    pltpu.VMEM((D, D), BF16),
    pltpu.VMEM((D, D), BF16),
    pltpu.VMEM((D, D), BF16),
    pltpu.VMEM((FF, D), BF16),
    pltpu.VMEM((FF, D), BF16),
    pltpu.VMEM((D,), BF16),
    pltpu.VMEM((1, D), F32),
    pltpu.VMEM((NT, S + 2 * HALO, 128), F32),
    pltpu.VMEM((D, D), F32),
    pltpu.VMEM((PADROWS, 128), F32),
    pltpu.VMEM((NT, PADROWS, 128), F32),
    pltpu.VMEM((NT, 128 * (NT + 1), 128), F32),
    pltpu.VMEM((D, D), BF16),
    pltpu.VMEM((D, D), BF16),
    pltpu.VMEM((1, D), F32),
    pltpu.VMEM((D, RL), BF16),
    pltpu.VMEM((S, D), BF16),
    pltpu.SemaphoreType.DMA((7,)),
    pltpu.SemaphoreType.DMA((len(WK_PIECES),)),
    pltpu.SemaphoreType.DMA((NT + 1,)),
    pltpu.SemaphoreType.DMA((NXC,)),
    pltpu.SemaphoreType.DMA((N2,)),
]


@jax.jit
def pallas_gated_mix__linear_attn_block__mixer_s_mlp__prompt_kernel(
    A_x: jax.Array,
    A_wqkv: jax.Array,
    A_wo: jax.Array,
    B_x: jax.Array,
    B_w1: jax.Array,
    B_w2: jax.Array,
    B_w3: jax.Array,
    B_w4: jax.Array,
    gate_w: jax.Array,
):
    del B_x
    return pl.pallas_call(
        _kernel,
        out_shape=jax.ShapeDtypeStruct((1, S, D), BF16),
        in_specs=[pl.BlockSpec(memory_space=pl.ANY)] * 8,
        out_specs=pl.BlockSpec(memory_space=pl.ANY),
        scratch_shapes=_SCRATCH,
        compiler_params=pltpu.CompilerParams(vmem_limit_bytes=100 * 2**20),
    )(A_x, A_wqkv, A_wo, B_w1, B_w2, B_w3.T, B_w4, gate_w)
```
